```python
import jax
import jax.numpy as jnp

def _softmax(x, axis=-1):
    return jax.nn.softmax(x, axis=axis)
def _gelu(x):
    return jax.nn.gelu(x, approximate=True)
def _silu(x):
    return jax.nn.silu(x)
def _sigmoid(x):
    return jax.nn.sigmoid(x)
def _layernorm(x, axis=-1, eps=1e-5):
    m = jnp.mean(x, axis=axis, keepdims=True)
    v = jnp.var(x, axis=axis, keepdims=True)
    return (x - m) / jnp.sqrt(v + eps)
def _scatter_add(tgt, idx, src, axis=0):
    return tgt.at[idx].add(src)
def _segment_sum(src, seg, n):
    return jax.ops.segment_sum(src, seg, n)
class _Rng:
    def __init__(self, key):
        self._k = key
    def _next(self):
        self._k, sub = jax.random.split(self._k)
        return sub
    def normal(self, shape):
        return jax.random.normal(self._next(), shape, dtype=jnp.bfloat16)
    def randint(self, lo, hi, shape):
        return jax.random.randint(self._next(), shape, lo, hi, dtype=jnp.int32)
    def uniform(self, shape, lo=0.0, hi=1.0):
        return jax.random.uniform(self._next(), shape, jnp.bfloat16, lo, hi)
    def permutation(self, n):
        return jax.random.permutation(self._next(), n)


kernel_name = 'gated_mix__sliding_block_cached__moe_arch_mod__decode'

def setup_inputs():
    _rng = _Rng(jax.random.key(int.from_bytes(__import__("os").urandom(4), "little")))
    _w = (lambda a: (lambda t: t.astype(jnp.bfloat16) if jnp.issubdtype(t.dtype, jnp.floating) else t)(jnp.asarray(a)))
    def _A_setup():
        B, Sq, D = 1, 1, 640
        Hq, Hkv, Sk, Dh = 32, 32, 32768, 192
        assert Hq % Hkv == 0, (Hq, Hkv)
        return {
            "x": _w((lambda *s: _rng.normal(s) * 0.05)(B, Sq, D)),
            "k_cache": _w((lambda *s: _rng.normal(s) * 0.05)(B, Hkv, Sk, Dh)),
            "v_cache": _w((lambda *s: _rng.normal(s) * 0.05)(B, Hkv, Sk, Dh)),
            "wq": _w((lambda *s: _rng.normal(s) * 0.05)(D, Hq * Dh) * (D ** -0.5)),
            "wo": _w((lambda *s: _rng.normal(s) * 0.05)(Hq * Dh, D) * ((Hq * Dh) ** -0.5)),
        }
    _A_in = _A_setup()

    def _B_setup():
        B, S, D, F, C = 1, 1, 640, 1536, 1
        return {
            "x": _w((lambda *s: _rng.normal(s) * 0.05)(B, S, D)),
            "w_r": _w((lambda *s: _rng.normal(s) * 0.05)(D)),
            "w_gate": _w((lambda *s: _rng.normal(s) * 0.05)(D, F)),
            "w_up": _w((lambda *s: _rng.normal(s) * 0.05)(D, F)),
            "w_down": _w((lambda *s: _rng.normal(s) * 0.05)(F, D)),
        }
    _B_in = _B_setup()

    return {
        "A_x": _A_in["x"],
        "A_k_cache": _A_in["k_cache"],
        "A_v_cache": _A_in["v_cache"],
        "A_wq": _A_in["wq"],
        "A_wo": _A_in["wo"],
        "B_x": _B_in["x"],
        "B_w_r": _B_in["w_r"],
        "B_w_gate": _B_in["w_gate"],
        "B_w_up": _B_in["w_up"],
        "B_w_down": _B_in["w_down"],
        "gate_w": _w((lambda *s: _rng.normal(s) * 0.05)(640)),
    }

def reference(A_x, A_k_cache, A_v_cache, A_wq, A_wo, B_x, B_w_r, B_w_gate, B_w_up, B_w_down, gate_w):
    def _A_ref(x, k_cache, v_cache, wq, wo):
        B, Sq, D = x.shape
        Hq, Dh = 32, 192
        Hkv, Sk = k_cache.shape[1], k_cache.shape[2]
        W = min(4096, max(256, Sk // 4))
        rep = Hq // Hkv
        q = (lambda x, *d: x.transpose(*d))((x @ wq).reshape(B, Sq, Hq, Dh), 0, 2, 1, 3)
        k = jnp.repeat(k_cache[:, :, Sk - W:, :], rep, axis=1)
        v = jnp.repeat(v_cache[:, :, Sk - W:, :], rep, axis=1)
        scores = jnp.einsum("bhqd,bhkd->bhqk", q, k) * (Dh ** -0.5)
        p = _softmax(scores, axis=-1)
        o = jnp.einsum("bhqk,bhkd->bhqd", p, v)
        return (lambda x, *d: x.transpose(*d))(o, 0, 2, 1, 3).reshape(B, Sq, Hq * Dh) @ wo

    def _B_ref(x, w_r, w_gate, w_up, w_down):
        B, S, D = x.shape
        C = 1
        r = x @ w_r
        idx = jnp.argsort(-r, axis=-1)[:, :C]
        idx_e = jnp.repeat(idx.reshape(B, C, 1), D, axis=2)
        x_sel = jnp.take_along_axis(x, idx_e, axis=1)
        g = _silu(x_sel @ w_gate)
        u = x_sel @ w_up
        y = (g * u) @ w_down
        r_sel = _sigmoid(jnp.take_along_axis(r, idx, axis=1))
        y = y * r_sel.reshape(B, C, 1)
        b_off = (jnp.arange(B) * S).reshape(B, 1)
        flat_idx = (idx + b_off).reshape(B * C)
        zero = (x * 0.0).reshape(B * S, D)
        upd = _scatter_add(zero, flat_idx, y.reshape(B * C, D), axis=0)
        return x + upd.reshape(B, S, D)

    x = A_x
    g = _sigmoid((x * gate_w).sum(-1, keepdims=True))
    a = _A_ref(x, A_k_cache, A_v_cache, A_wq, A_wo)
    b = _B_ref(x, B_w_r, B_w_gate, B_w_up, B_w_down)
    return g * a + (1 - g) * b
```

```python
import functools

import jax
import jax.numpy as jnp
import jax.experimental.pallas as pl
import jax.experimental.pallas.tpu as pltpu

_HQ = 32
_DH = 192
_GROUP = 8
_GROWS = _GROUP * _DH


def _kernel(x_hbm, k_hbm, v_hbm, wq_hbm, wo_hbm, wr_hbm, wg_hbm, wu_hbm, wd_hbm, gw_hbm,
            o_ref,
            x_buf, small_buf, wq_buf, wo_buf, wg_buf, wu_buf, wd_buf, kv_buf,
            q_buf, s_buf, p_buf, acc_buf,
            sem_small, sem_wq, sem_w, sem_wd, sem_kv,
            *, R, NB, W, SK, D, F, WD_CHUNK):
    f32, bf16 = jnp.float32, jnp.bfloat16
    n_rows = _HQ * _DH
    NC = n_rows // R
    SUB = _GROWS // R
    NG = _HQ // _GROUP
    NWD = F // WD_CHUNK
    col0 = SK - W

    def kv_copy(src, row, slot):
        return pltpu.make_async_copy(
            src.at[pl.ds(row, R), pl.ds(col0, W)], kv_buf.at[slot], sem_kv.at[slot])

    def wq_copy(g):
        return pltpu.make_async_copy(
            wq_hbm.at[:, pl.ds(g * _GROWS, _GROWS)], wq_buf.at[g], sem_wq.at[g])

    def wd_copy(c):
        return pltpu.make_async_copy(
            wd_hbm.at[pl.ds(c * WD_CHUNK, WD_CHUNK), :], wd_buf.at[c], sem_wd.at[c])

    x_cp = pltpu.make_async_copy(x_hbm, x_buf, sem_small.at[0])
    wr_cp = pltpu.make_async_copy(wr_hbm, small_buf.at[0], sem_small.at[1])
    gw_cp = pltpu.make_async_copy(gw_hbm, small_buf.at[1], sem_small.at[2])
    wg_cp = pltpu.make_async_copy(wg_hbm, wg_buf, sem_w.at[0])
    wu_cp = pltpu.make_async_copy(wu_hbm, wu_buf, sem_w.at[1])
    wo_cp = pltpu.make_async_copy(wo_hbm, wo_buf, sem_w.at[2])

    wq_copy(0).start()
    x_cp.start()
    for g in range(1, NG):
        wq_copy(g).start()
    wr_cp.start()
    gw_cp.start()
    for j in range(NB):
        kv_copy(k_hbm, j * R, j).start()
    wg_cp.start()
    wu_cp.start()
    wo_cp.start()

    x_cp.wait()
    x_row = x_buf[...]
    x8 = jnp.broadcast_to(x_row.astype(f32), (8, D)).astype(bf16)

    row_id = jax.lax.broadcasted_iota(jnp.int32, (8, _GROWS), 0)
    col_id = jax.lax.broadcasted_iota(jnp.int32, (8, _GROWS), 1)
    bd = jnp.logical_and(col_id >= row_id * _DH, col_id < (row_id + 1) * _DH)

    def q_body(g, c):
        wq_copy(g).wait()
        q = jnp.dot(x8, wq_buf[g], preferred_element_type=f32)
        q = jnp.where(bd, q, 0.0)
        for s in range(SUB):
            q_buf[g * SUB + s] = q[:, s * R:(s + 1) * R]
        return c
    jax.lax.fori_loop(0, NG, q_body, 0)

    def start_next(j):
        nxt = j + NB
        slot = j % NB

        @pl.when(nxt < NC)
        def _():
            kv_copy(k_hbm, pl.multiple_of(nxt * R, R), slot).start()

        @pl.when(jnp.logical_and(nxt >= NC, nxt < 2 * NC))
        def _():
            kv_copy(v_hbm, pl.multiple_of((nxt - NC) * R, R), slot).start()

    s_buf[...] = jnp.zeros(s_buf.shape, f32)

    def k_body(j, c):
        slot = j % NB
        kv_copy(k_hbm, 0, slot).wait()
        g = j // SUB
        s = jnp.dot(q_buf[j].astype(bf16), kv_buf[slot], preferred_element_type=f32)
        s_buf[g] += s
        start_next(j)
        return c
    jax.lax.fori_loop(0, NC, k_body, 0)

    scale = _DH ** -0.5
    for g in range(NG):
        s = s_buf[g] * scale
        m = jnp.max(s, axis=-1, keepdims=True)
        e = jnp.exp(s - m)
        l = jnp.sum(e, axis=-1, keepdims=True)
        p_buf[g] = e / l

    wg_cp.wait()
    wu_cp.wait()
    hg = jnp.dot(x8, wg_buf[...], preferred_element_type=f32)
    hu = jnp.dot(x8, wu_buf[...], preferred_element_type=f32)
    h = (jax.nn.silu(hg) * hu).astype(bf16)

    wr_cp.wait()
    gw_cp.wait()
    xf = x_row.astype(f32)
    wr = small_buf[0].astype(f32)
    gw = small_buf[1].astype(f32)
    r_acc = jnp.zeros((1, 128), f32)
    g_acc = jnp.zeros((1, 128), f32)
    for t in range(D // 128):
        xt = xf[:, t * 128:(t + 1) * 128]
        r_acc = r_acc + xt * wr[t:t + 1, :]
        g_acc = g_acc + xt * gw[t:t + 1, :]
    r_sel = jax.nn.sigmoid(jnp.sum(r_acc, axis=-1, keepdims=True))
    gate = jax.nn.sigmoid(jnp.sum(g_acc, axis=-1, keepdims=True))

    wo_cp.wait()
    acc_buf[...] = jnp.zeros(acc_buf.shape, f32)
    rowc = jax.lax.broadcasted_iota(jnp.int32, (8, R), 0)
    colc = jax.lax.broadcasted_iota(jnp.int32, (8, R), 1)

    def v_body(jj, c):
        j = jj + NC
        slot = j % NB
        kv_copy(v_hbm, 0, slot).wait()
        g = jj // SUB
        sub = jj % SUB
        o = jax.lax.dot_general(p_buf[g].astype(bf16), kv_buf[slot],
                                (((1,), (1,)), ((), ())), preferred_element_type=f32)
        cg = colc + sub * R
        msk = jnp.logical_and(cg >= rowc * _DH, cg < (rowc + 1) * _DH)
        o = jnp.where(msk, o, 0.0).astype(bf16)
        wo = wo_buf[pl.ds(pl.multiple_of(jj * R, R), R), :]
        acc_buf[...] += jnp.dot(o, wo, preferred_element_type=f32)
        start_next(j)

        @pl.when(j + NB == 2 * NC)
        def _():
            for cc in range(NWD):
                wd_copy(cc).start()
        return c
    jax.lax.fori_loop(0, NC, v_body, 0)

    a = jnp.sum(acc_buf[...], axis=0, keepdims=True)

    y = jnp.zeros((8, D), f32)
    for cc in range(NWD):
        wd_copy(cc).wait()
        y = y + jnp.dot(h[:, cc * WD_CHUNK:(cc + 1) * WD_CHUNK], wd_buf[cc],
                        preferred_element_type=f32)
    y = y[0:1, :] * r_sel
    b = xf + (xf * 0.0 + y)
    o_ref[...] = (gate * a + (1.0 - gate) * b).astype(o_ref.dtype)


def _build(R=384, NB=4, WD_CHUNK=256):
    def fn(A_x, A_k_cache, A_v_cache, A_wq, A_wo, B_x, B_w_r, B_w_gate, B_w_up, B_w_down, gate_w):
        B, Sq, D = A_x.shape
        _, Hkv, SK, Dh = A_k_cache.shape
        assert B == 1 and Sq == 1 and Hkv == _HQ and Dh == _DH
        W = min(4096, max(256, SK // 4))
        F = B_w_gate.shape[1]
        n_rows = _HQ * _DH
        NC = n_rows // R
        bf16, f32 = jnp.bfloat16, jnp.float32

        x = A_x.reshape(1, D)
        kt = jnp.swapaxes(A_k_cache, 2, 3).reshape(n_rows, SK)
        vt = jnp.swapaxes(A_v_cache, 2, 3).reshape(n_rows, SK)
        wr = B_w_r.reshape(D // 128, 128)
        gw = gate_w.reshape(D // 128, 128)

        any_spec = pl.BlockSpec(memory_space=pl.ANY)
        out = pl.pallas_call(
            functools.partial(_kernel, R=R, NB=NB, W=W, SK=SK, D=D, F=F, WD_CHUNK=WD_CHUNK),
            in_specs=[any_spec] * 10,
            out_specs=pl.BlockSpec(memory_space=pltpu.VMEM),
            out_shape=jax.ShapeDtypeStruct((1, D), bf16),
            scratch_shapes=[
                pltpu.VMEM((1, D), bf16),
                pltpu.VMEM((2, D // 128, 128), bf16),
                pltpu.VMEM((_HQ // _GROUP, D, _GROWS), bf16),
                pltpu.VMEM((n_rows, D), bf16),
                pltpu.VMEM((D, F), bf16),
                pltpu.VMEM((D, F), bf16),
                pltpu.VMEM((F // WD_CHUNK, WD_CHUNK, D), bf16),
                pltpu.VMEM((NB, R, W), bf16),
                pltpu.VMEM((NC, 8, R), f32),
                pltpu.VMEM((_HQ // _GROUP, 8, W), f32),
                pltpu.VMEM((_HQ // _GROUP, 8, W), f32),
                pltpu.VMEM((8, D), f32),
                pltpu.SemaphoreType.DMA((3,)),
                pltpu.SemaphoreType.DMA((_HQ // _GROUP,)),
                pltpu.SemaphoreType.DMA((3,)),
                pltpu.SemaphoreType.DMA((F // WD_CHUNK,)),
                pltpu.SemaphoreType.DMA((NB,)),
            ],
            compiler_params=pltpu.CompilerParams(vmem_limit_bytes=100 * 1024 * 1024),
        )(x, kt, vt, A_wq, A_wo, wr, B_w_gate, B_w_up, B_w_down, gw)
        return out.reshape(B, Sq, D)
    return fn


@jax.jit
def pallas_gated_mix__sliding_block_cached__moe_arch_mod__decode_kernel(
    A_x: jax.Array,
    A_k_cache: jax.Array,
    A_v_cache: jax.Array,
    A_wq: jax.Array,
    A_wo: jax.Array,
    B_x: jax.Array,
    B_w_r: jax.Array,
    B_w_gate: jax.Array,
    B_w_up: jax.Array,
    B_w_down: jax.Array,
    gate_w: jax.Array,
):
    return _build()(A_x, A_k_cache, A_v_cache, A_wq, A_wo, B_x, B_w_r,
                    B_w_gate, B_w_up, B_w_down, gate_w)
```

```python
import dataclasses
import functools

import jax
import jax.numpy as jnp
import jax.experimental.pallas as pl
import jax.experimental.pallas.tpu as pltpu

_HQ = 32
_DH = 192
_PR = 2 * _DH
_NP = _HQ // 2
_LN = 128


def _const_div(n, d, hi):
    for sh in range(1, 20):
        m = -(-(1 << sh) // d)
        if all((v * m) >> sh == v // d for v in range(hi)):
            return jax.lax.shift_right_logical(n * m, sh)
    raise ValueError("no multiplier")


def _compiler_params(**kw):
    names = {f.name for f in dataclasses.fields(pltpu.CompilerParams)}
    return pltpu.CompilerParams(**{k: v for k, v in kw.items() if k in names})


def _kernel(x_hbm, k_hbm, v_hbm, wq_hbm, wo_hbm, wr_hbm, wg_hbm, wu_hbm, wd_hbm, gw_hbm,
            o_ref,
            x_buf, small_buf, wq_buf, wgu_buf, wo_buf, ring,
            x8_buf, q_buf, s_buf, m_buf, ob_buf, h_buf, a_buf, y_buf,
            sem_small, sem_wq, sem_gu, sem_wo, sem_ring,
            *, D1, D0, W, SK, D, F, VS, UNR):
    f32, bf16 = jnp.float32, jnp.bfloat16
    NC = W // _LN
    NS = _NP * NC
    DB = D // _LN
    FB = F // _LN
    PB = _PR // _LN
    HT = 64
    col0 = SK - W
    NWD = (F // _PR) * DB
    assert NC == 32 and D1 < NC and D % _LN == 0 and F % _PR == 0
    PRE = 2
    QH = D // HT
    assert QH == 2 * DB
    N_WQ = (_NP - PRE) * PB * QH
    N_GU = FB * 2 * DB
    OH = _PR // HT
    N_WO = _NP * DB * OH
    S_GU = N_WQ
    S_WO = S_GU + N_GU
    S_WD = S_WO + N_WO
    assert S_GU <= NS <= S_WO and S_WD + D0 == 2 * NS
    WD1 = _PR - HT
    scale = _DH ** -0.5
    VR = _PR // VS

    mo = pl.multiple_of

    def kv_start(src, t):
        row = mo(jax.lax.shift_right_logical(t, 5) * _PR, _PR)
        c = jnp.bitwise_and(t, NC - 1)
        col = mo(col0 + c * _LN, _LN)
        pltpu.make_async_copy(src.at[pl.ds(row, _PR), pl.ds(col, _LN)],
                              ring.at[c], sem_ring.at[c]).start(priority=1)

    def wd_start(i, part):
        row = jnp.bitwise_and(i, 3) * _PR
        col = mo(jax.lax.shift_right_logical(i, 2) * _LN, _LN)
        if part == 1:
            pltpu.make_async_copy(wd_hbm.at[pl.ds(mo(row, HT), WD1), pl.ds(col, _LN)],
                                  ring.at[i, pl.ds(0, WD1)], sem_ring.at[i]).start(priority=1)
        else:
            pltpu.make_async_copy(wd_hbm.at[pl.ds(mo(row + WD1, HT), HT), pl.ds(col, _LN)],
                                  ring.at[i, pl.ds(WD1, HT)], sem_ring.at[i]).start(priority=0)

    def ring_wait(c):
        pltpu.make_async_copy(ring.at[c], ring.at[c], sem_ring.at[c]).wait()

    def wq_gu_start(n, with_wq):
        u = n + PRE * PB * QH
        cb = _const_div(u, QH, 1100)
        t = u - cb * QH
        if with_wq:
            @pl.when(n < S_GU)
            def _():
                pair = _const_div(cb, PB, 128)
                pltpu.make_async_copy(
                    wq_hbm.at[pl.ds(mo(t * HT, HT), HT), pl.ds(mo(cb * _LN, _LN), _LN)],
                    wq_buf.at[cb, pl.ds(mo(t * HT, HT), HT)], sem_wq.at[pair]).start(priority=0)
        ch = cb - _NP * PB
        in_gu = jnp.logical_and(n >= S_GU, n < S_WO)

        @pl.when(jnp.logical_and(in_gu, t < DB))
        def _():
            pltpu.make_async_copy(
                wg_hbm.at[pl.ds(mo(t * _LN, _LN), _LN), pl.ds(mo(ch * _LN, _LN), _LN)],
                wgu_buf.at[ch, pl.ds(mo(t * _LN, _LN), _LN)], sem_gu.at[ch]).start(priority=0)

        @pl.when(jnp.logical_and(in_gu, t >= DB))
        def _():
            pltpu.make_async_copy(
                wu_hbm.at[pl.ds(mo((t - DB) * _LN, _LN), _LN), pl.ds(mo(ch * _LN, _LN), _LN)],
                wgu_buf.at[ch, pl.ds(mo(t * _LN, _LN), _LN)], sem_gu.at[ch]).start(priority=0)

    def wo_start(n):
        @pl.when(jnp.logical_and(n >= S_WO, n < S_WD))
        def _():
            w = n - S_WO
            jj = _const_div(w, OH, N_WO)
            r = w - jj * OH
            pair = _const_div(jj, DB, 128)
            cb = jj - pair * DB
            pltpu.make_async_copy(
                wo_hbm.at[pl.ds(mo(pair * _PR + r * HT, HT), HT), pl.ds(mo(cb * _LN, _LN), _LN)],
                wo_buf.at[jj, pl.ds(mo(r * HT, HT), HT)], sem_wo.at[pair]).start(priority=0)

    def wq_wait(pair):
        blk = wq_buf.at[pl.ds(pair * PB, PB)]
        pltpu.make_async_copy(blk, blk, sem_wq.at[pair]).wait()

    def wo_wait(pair):
        blk = wo_buf.at[pl.ds(pair * DB, DB)]
        pltpu.make_async_copy(blk, blk, sem_wo.at[pair]).wait()

    x_cp = pltpu.make_async_copy(x_hbm, x_buf, sem_small.at[0])
    wr_cp = pltpu.make_async_copy(wr_hbm, small_buf.at[0], sem_small.at[1])
    gw_cp = pltpu.make_async_copy(gw_hbm, small_buf.at[1], sem_small.at[2])

    def wq_pre(cb):
        pltpu.make_async_copy(wq_hbm.at[:, pl.ds(cb * _LN, _LN)], wq_buf.at[cb],
                              sem_wq.at[cb // PB]).start(priority=0)
    wq_pre(0)
    x_cp.start(priority=0)
    for cb in range(1, PRE * PB):
        wq_pre(cb)
    wr_cp.start(priority=0)
    gw_cp.start(priority=0)
    for j in range(D1):
        pltpu.make_async_copy(k_hbm.at[pl.ds(0, _PR), pl.ds(col0 + j * _LN, _LN)],
                              ring.at[j], sem_ring.at[j]).start(priority=1)

    x_cp.wait()
    xf = x_buf[...].astype(f32)
    x8_buf[...] = jnp.broadcast_to(xf, (8, D))
    a_buf[...] = jnp.zeros(a_buf.shape, f32)
    y_buf[...] = jnp.zeros(y_buf.shape, f32)

    row_id = jax.lax.broadcasted_iota(jnp.int32, (8, _LN), 0)
    lane_id = jax.lax.broadcasted_iota(jnp.int32, (8, _LN), 1)

    def head_mask(k):
        col = lane_id + k * _LN
        return jnp.logical_and(col >= row_id * _DH, col < (row_id + 1) * _DH)

    def q_job(cb, k):
        q = jnp.dot(x8_buf[...].astype(bf16), wq_buf[cb], preferred_element_type=f32)
        q_buf[cb] = jnp.where(head_mask(k), q, 0.0)

    wq_wait(0)
    for k in range(PB):
        q_job(k, k)

    wr_cp.wait()
    gw_cp.wait()
    wr = small_buf[0].astype(f32)
    gw = small_buf[1].astype(f32)
    r_acc = jnp.zeros((1, _LN), f32)
    g_acc = jnp.zeros((1, _LN), f32)
    for t in range(DB):
        xt = xf[:, t * _LN:(t + 1) * _LN]
        r_acc = r_acc + xt * wr[t:t + 1, :]
        g_acc = g_acc + xt * gw[t:t + 1, :]
    r_sel = jax.nn.sigmoid(jnp.sum(r_acc, axis=-1, keepdims=True))
    gate = jax.nn.sigmoid(jnp.sum(g_acc, axis=-1, keepdims=True))

    def cat(buf, base, n):
        return jnp.concatenate([buf[base + k] for k in range(n)], axis=1).astype(bf16)

    def k_slot(p, c, m, job=None):
        n = p * NC + c
        ring_wait(c)
        s = jnp.dot(cat(q_buf, p * PB, PB), ring[c], preferred_element_type=f32)
        if job is not None:
            job()
        wq_gu_start(n, True)
        t = n + D1

        @pl.when(t < NS)
        def _():
            kv_start(k_hbm, t)

        @pl.when(t >= NS)
        def _():
            kv_start(v_hbm, t - NS)
        s_buf[n] = s
        return jnp.maximum(m, s)

    def k_period(p, carry):
        na = jnp.where(p < _NP - 1, PB, 0)
        m = jnp.full((8, _LN), -jnp.inf, f32)
        m = jax.lax.fori_loop(0, NC - na, lambda c, m: k_slot(p, c, m), m)

        @pl.when(p < _NP - 1)
        def _():
            wq_wait(p + 1)

        def body(c, m):
            k = c - (NC - PB)
            return k_slot(p, c, m, lambda: q_job((p + 1) * PB + k, k))
        m = jax.lax.fori_loop(NC - na, NC, body, m)
        m_buf[p] = jnp.broadcast_to(jnp.max(m, axis=-1, keepdims=True), (8, _LN))
        return carry
    jax.lax.fori_loop(0, _NP, k_period, 0)

    def prob(n):
        return jnp.exp((s_buf[n] - m_buf[jax.lax.shift_right_logical(n, 5)]) * scale)

    def v_slot(p, c, st, job=None):
        e, l, o = st
        nn = p * NC + c
        n = nn + NS
        ring_wait(c)
        eb = e.astype(bf16)
        pv = [jax.lax.dot_general(eb, ring[c, pl.ds(k * VR, VR), :], (((1,), (1,)), ((), ())),
                                  preferred_element_type=f32) for k in range(VS)]
        if job is not None:
            job()
        wq_gu_start(n, False)
        wo_start(n)

        @pl.when(n >= S_WD)
        def _():
            wd_start(n - S_WD, 0)
        t = nn + D1

        @pl.when(t < NS)
        def _():
            kv_start(v_hbm, t)

        @pl.when(jnp.logical_and(t >= NS, t < NS + NWD))
        def _():
            wd_start(t - NS, 1)
        l = l + e
        e = prob(jnp.minimum(nn + 1, NS - 1))
        return e, l, tuple(a + b for a, b in zip(o, pv))

    def o_job(pair, cb):
        acc = a_buf[cb]
        for k in range(VS):
            acc = acc + jnp.dot(ob_buf[pair * VS + k].astype(bf16),
                                wo_buf[pair * DB + cb, pl.ds(k * VR, VR), :],
                                preferred_element_type=f32)
        a_buf[cb] = acc

    def ffn_job(ch):
        x8 = x8_buf[...].astype(bf16)
        hg = jnp.dot(x8, wgu_buf[ch, pl.ds(0, D)], preferred_element_type=f32)
        hu = jnp.dot(x8, wgu_buf[ch, pl.ds(D, D)], preferred_element_type=f32)
        h_buf[ch] = jax.nn.silu(hg) * hu

    LAG = 2

    def v_period(p, e):
        na = jnp.where(p >= LAG, DB, 0)
        nb = jnp.where(p < FB, 1, 0)
        st = (e, jnp.zeros((8, _LN), f32), tuple(jnp.zeros((8, VR), f32) for _ in range(VS)))
        st = jax.lax.fori_loop(0, NC - na - nb, lambda c, st: v_slot(p, c, st), st)

        @pl.when(p < FB)
        def _():
            blk = wgu_buf.at[p]
            pltpu.make_async_copy(blk, blk, sem_gu.at[p]).wait()

        def body_b(c, st):
            return v_slot(p, c, st, lambda: ffn_job(p))
        st = jax.lax.fori_loop(NC - na - nb, NC - na, body_b, st)

        @pl.when(p >= LAG)
        def _():
            wo_wait(p - LAG)

        def body_a(c, st):
            return v_slot(p, c, st, lambda: o_job(p - LAG, c - (NC - DB)))
        e, l, o = jax.lax.fori_loop(NC - na, NC, body_a, st)
        inv = 1.0 / jnp.sum(l, axis=-1, keepdims=True)
        rr = jax.lax.broadcasted_iota(jnp.int32, (8, VR), 0)
        cc = jax.lax.broadcasted_iota(jnp.int32, (8, VR), 1)
        for k in range(VS):
            col = cc + k * VR
            msk = jnp.logical_and(col >= rr * _DH, col < (rr + 1) * _DH)
            ob_buf[p * VS + k] = jnp.where(msk, o[k] * inv, 0.0)
        return e
    jax.lax.fori_loop(0, _NP, v_period, prob(0))

    def d_slot(i, job=None):
        ring_wait(i)
        cb = jax.lax.shift_right_logical(i, 2)
        y = jnp.dot(cat(h_buf, jnp.bitwise_and(i, 3) * PB, PB), ring[i],
                    preferred_element_type=f32)
        if job is not None:
            job()

        @pl.when(i + D0 < NWD)
        def _():
            wd_start(i + D0, 0)
        if D1 < NWD:
            @pl.when(i + D1 < NWD)
            def _():
                wd_start(i + D1, 1)
        y_buf[cb] += y

    for pair in range(_NP - LAG, _NP):
        wo_wait(pair)
        base = (pair - (_NP - LAG)) * DB

        def body_d(i, carry, pair=pair, base=base):
            d_slot(i, lambda: o_job(pair, i - base))
            return carry
        jax.lax.fori_loop(base, base + DB, body_d, 0)

    a = jnp.concatenate([jnp.sum(a_buf[k], axis=0, keepdims=True) for k in range(DB)], axis=1)
    base_out = gate * a + (1.0 - gate) * (xf + xf * 0.0)
    cy = (1.0 - gate) * r_sel

    def body_e(i, carry):
        d_slot(i)
        return carry
    jax.lax.fori_loop(LAG * DB, NWD, body_e, 0)

    y = jnp.concatenate([y_buf[k][0:1, :] for k in range(DB)], axis=1)
    o_ref[...] = (base_out + cy * y).astype(o_ref.dtype)


def _build(D1=20, D0=4, VS=4, UNR=1):
    def fn(A_x, A_k_cache, A_v_cache, A_wq, A_wo, B_x, B_w_r, B_w_gate, B_w_up, B_w_down, gate_w):
        B, Sq, D = A_x.shape
        _, Hkv, SK, Dh = A_k_cache.shape
        assert B == 1 and Sq == 1 and Hkv == _HQ and Dh == _DH
        W = min(4096, max(256, SK // 4))
        F = B_w_gate.shape[1]
        n_rows = _HQ * _DH
        NC = W // _LN
        DB, FB, PB = D // _LN, F // _LN, _PR // _LN
        bf16, f32 = jnp.bfloat16, jnp.float32

        x = A_x.reshape(1, D)
        kt = jnp.swapaxes(A_k_cache, 2, 3).reshape(n_rows, SK)
        vt = jnp.swapaxes(A_v_cache, 2, 3).reshape(n_rows, SK)
        wr = B_w_r.reshape(DB, _LN)
        gw = gate_w.reshape(DB, _LN)

        any_spec = pl.BlockSpec(memory_space=pl.ANY)
        out = pl.pallas_call(
            functools.partial(_kernel, D1=D1, D0=D0, VS=VS, UNR=UNR, W=W, SK=SK, D=D, F=F),
            in_specs=[any_spec] * 10,
            out_specs=pl.BlockSpec(memory_space=pltpu.VMEM),
            out_shape=jax.ShapeDtypeStruct((1, D), bf16),
            scratch_shapes=[
                pltpu.VMEM((1, D), bf16),
                pltpu.VMEM((2, DB, _LN), bf16),
                pltpu.VMEM((_NP * PB, D, _LN), bf16),
                pltpu.VMEM((FB, 2 * D, _LN), bf16),
                pltpu.VMEM((_NP * DB, _PR, _LN), bf16),
                pltpu.VMEM((NC, _PR, _LN), bf16),
                pltpu.VMEM((8, D), f32),
                pltpu.VMEM((_NP * PB, 8, _LN), f32),
                pltpu.VMEM((_NP * NC, 8, _LN), f32),
                pltpu.VMEM((_NP, 8, _LN), f32),
                pltpu.VMEM((_NP * VS, 8, _PR // VS), f32),
                pltpu.VMEM((FB, 8, _LN), f32),
                pltpu.VMEM((DB, 8, _LN), f32),
                pltpu.VMEM((DB, 8, _LN), f32),
                pltpu.SemaphoreType.DMA((3,)),
                pltpu.SemaphoreType.DMA((_NP,)),
                pltpu.SemaphoreType.DMA((FB,)),
                pltpu.SemaphoreType.DMA((_NP,)),
                pltpu.SemaphoreType.DMA((NC,)),
            ],
            compiler_params=_compiler_params(vmem_limit_bytes=100 * 1024 * 1024,
                                             disable_bounds_checks=True,
                                             disable_semaphore_checks=True),
        )(x, kt, vt, A_wq, A_wo, wr, B_w_gate, B_w_up, B_w_down, gw)
        return out.reshape(B, Sq, D)
    return fn


@jax.jit
def pallas_gated_mix__sliding_block_cached__moe_arch_mod__decode_kernel(
    A_x: jax.Array,
    A_k_cache: jax.Array,
    A_v_cache: jax.Array,
    A_wq: jax.Array,
    A_wo: jax.Array,
    B_x: jax.Array,
    B_w_r: jax.Array,
    B_w_gate: jax.Array,
    B_w_up: jax.Array,
    B_w_down: jax.Array,
    gate_w: jax.Array,
):
    return _build()(A_x, A_k_cache, A_v_cache, A_wq, A_wo, B_x, B_w_r,
                    B_w_gate, B_w_up, B_w_down, gate_w)
```

```python
import dataclasses
import functools

import jax
import jax.numpy as jnp
import jax.experimental.pallas as pl
import jax.experimental.pallas.tpu as pltpu

_HQ = 32
_DH = 192
_PR = 2 * _DH
_NP = _HQ // 2
_LN = 128


def _const_div(n, d, hi):
    for sh in range(1, 20):
        m = -(-(1 << sh) // d)
        if all((v * m) >> sh == v // d for v in range(hi)):
            return jax.lax.shift_right_logical(n * m, sh)
    raise ValueError("no multiplier")


def _compiler_params(**kw):
    names = {f.name for f in dataclasses.fields(pltpu.CompilerParams)}
    return pltpu.CompilerParams(**{k: v for k, v in kw.items() if k in names})


class _NoScope:
    def __enter__(self):
        return self

    def __exit__(self, *a):
        return False


def _kernel(x_hbm, k_hbm, v_hbm, wq_hbm, wo_hbm, wr_hbm, wg_hbm, wu_hbm, wd_hbm, gw_hbm,
            o_ref,
            x_buf, small_buf, wq_buf, wgu_buf, wo_buf, wd_buf, ring,
            x8_buf, q_buf, s_buf, m_buf, ob_buf, l_buf, h_buf, a_buf, y_buf,
            sem_small, sem_wq, sem_gu, sem_wo, sem_wd, sem_ring,
            *, D1, W, SK, D, F, SCOPES, TAILP, TAILG, OC):
    f32, bf16 = jnp.float32, jnp.bfloat16
    scope = jax.named_scope if SCOPES else (lambda name: _NoScope())
    NC = W // _LN
    NS = _NP * NC
    DB = D // _LN
    FB = F // _LN
    PB = _PR // _LN
    VS = 4
    VR = _PR // VS
    HT = 64
    col0 = SK - W
    assert NC == 32 and D1 < NC and D % _LN == 0 and F % _LN == 0
    XS = NC // 2
    assert D1 + XS <= NC
    XR = 160
    XP = D // XR
    N_X = 2 * PB * XP
    N_WQ = (_NP - 2) * PB * DB
    GR = 8
    N_WG = D // GR
    UR, UC = 16, 4 * _LN
    UB = F // UC
    N_WU = (D // UR) * UB
    S_WQ = N_X
    S_WG = S_WQ + N_WQ
    S_WU = S_WG + N_WG
    S_D1 = S_WU + N_WU
    N_D1 = NS - S_D1
    OP = (_PR // HT) * DB
    N_WO = _NP * OP
    TAIL = 2
    CP = (_LN // HT) * DB
    N_WD = (FB - TAIL) * CP
    assert 0 < N_D1 <= N_WD and N_WO + N_WD - N_D1 <= NS
    WD_A = N_D1 // CP
    WD_B = FB - TAIL
    S_D2 = N_WO - OP
    N_D2 = N_WD - N_D1
    scale = _DH ** -0.5

    mo = pl.multiple_of
    srl = jax.lax.shift_right_logical

    def kv_start(src, t):
        row = mo(srl(t, 5) * _PR, _PR)
        c = jnp.bitwise_and(t, NC - 1)
        col = mo(col0 + c * _LN, _LN)
        pltpu.make_async_copy(src.at[pl.ds(row, _PR), pl.ds(col, _LN)],
                              ring.at[c], sem_ring.at[c]).start(priority=1)

    def wait_all(ref, sem):
        pltpu.make_async_copy(ref, ref, sem).wait()

    def band_start(src, dst, u, sem):
        band = _const_div(u, DB, 520)
        row = mo(band * HT, HT)
        col = mo((u - band * DB) * _LN, _LN)
        pltpu.make_async_copy(src.at[pl.ds(row, HT), pl.ds(col, _LN)],
                              dst.at[pl.ds(row, HT), pl.ds(col, _LN)], sem).start(priority=0)

    def wd_start(u):
        idx = (u >= WD_A * CP).astype(jnp.int32)
        band_start(wd_hbm, wd_buf, u, sem_wd.at[idx])

    def early_start(n):
        cb = srl(n, 2)
        row = mo(jnp.bitwise_and(n, XP - 1) * XR, 16)
        pltpu.make_async_copy(
            wq_hbm.at[pl.ds(row, XR), pl.ds(mo(cb * _LN, _LN), _LN)],
            wq_buf.at[cb, pl.ds(row, XR)],
            sem_wq.at[(n >= PB * XP).astype(jnp.int32)]).start(priority=0)

    def wq_start(n):
        u = n - S_WQ + 2 * PB * DB
        cb = _const_div(u, DB, NS + 2 * PB * DB)
        row = mo((u - cb * DB) * _LN, _LN)
        pltpu.make_async_copy(
            wq_hbm.at[pl.ds(row, _LN), pl.ds(mo(cb * _LN, _LN), _LN)],
            wq_buf.at[cb, pl.ds(row, _LN)], sem_wq.at[_const_div(cb, PB, 128)]).start(priority=0)

    def k_phase_start(n):
        @pl.when(n < S_WG)
        def _():
            wq_start(n)

        @pl.when(jnp.logical_and(n >= S_WG, n < S_WU))
        def _():
            row = mo((n - S_WG) * GR, GR)
            pltpu.make_async_copy(wg_hbm.at[pl.ds(row, GR)], wgu_buf.at[0, pl.ds(row, GR)],
                                  sem_gu.at[0]).start(priority=0)

        @pl.when(jnp.logical_and(n >= S_WU, n < S_D1))
        def _():
            u = n - S_WU
            r = _const_div(u, UB, NS)
            sl = (pl.ds(mo(r * UR, UR), UR), pl.ds(mo((u - r * UB) * UC, _LN), UC))
            pltpu.make_async_copy(wu_hbm.at[sl], wgu_buf.at[1].at[sl],
                                  sem_gu.at[0]).start(priority=0)

        @pl.when(n >= S_D1)
        def _():
            wd_start(n - S_D1)
        t = n + D1

        @pl.when(t < NS)
        def _():
            kv_start(k_hbm, t)

        @pl.when(t >= NS)
        def _():
            kv_start(v_hbm, t - NS)

    tail_parts = TAILP

    def tail_copy(i):
        ch, c0, cn = tail_parts[i]
        sl = (pl.ds(ch * _LN, _LN), pl.ds(c0 * _LN, cn * _LN))
        return pltpu.make_async_copy(wd_hbm.at[sl], wd_buf.at[sl], sem_wd.at[2 + i])

    def v_phase_start(n):
        in_wd = jnp.logical_and(n >= S_D2, n < S_D2 + N_D2)

        @pl.when(jnp.logical_and(jnp.logical_not(in_wd), n < N_WO + N_D2))
        def _():
            u = jnp.where(n < S_D2, n, n - N_D2)
            band_start(wo_hbm, wo_buf, u, sem_wo.at[_const_div(u, OP, NS)])

        @pl.when(in_wd)
        def _():
            wd_start(n - S_D2 + N_D1)
        t = n + D1

        @pl.when(t < NS)
        def _():
            kv_start(v_hbm, t)

        @pl.when(t == NS)
        def _():
            for i in range(len(tail_parts)):
                tail_copy(i).start(priority=1)

    x_cp = pltpu.make_async_copy(x_hbm, x_buf, sem_small.at[0])
    wr_cp = pltpu.make_async_copy(wr_hbm, small_buf.at[0], sem_small.at[1])
    gw_cp = pltpu.make_async_copy(gw_hbm, small_buf.at[1], sem_small.at[2])
    for j in range(D1):
        pltpu.make_async_copy(k_hbm.at[pl.ds(0, _PR), pl.ds(col0 + j * _LN, _LN)],
                              ring.at[j], sem_ring.at[j]).start(priority=1)
    x_cp.start(priority=0)
    wr_cp.start(priority=0)
    gw_cp.start(priority=0)

    def x0_slot(n, carry):
        wait_all(ring.at[n], sem_ring.at[n])
        early_start(n)
        kv_start(k_hbm, n + D1)
        return carry
    with scope("x0"):
        jax.lax.fori_loop(0, XS, x0_slot, 0)

    x_cp.wait()
    xf = x_buf[...].astype(f32)
    x8_buf[...] = jnp.broadcast_to(xf, (8, D))
    a_buf[...] = jnp.zeros(a_buf.shape, f32)
    y_buf[...] = jnp.zeros(y_buf.shape, f32)

    row_id = jax.lax.broadcasted_iota(jnp.int32, (8, _LN), 0)
    lane_id = jax.lax.broadcasted_iota(jnp.int32, (8, _LN), 1)

    def q_job(pair, k):
        q = jnp.dot(x8_buf[...].astype(bf16), wq_buf[pair * PB + k], preferred_element_type=f32)
        hc = lane_id + k * _LN
        own = jnp.logical_and(hc >= row_id * _DH, hc < (row_id + 1) * _DH)
        q_buf[pair * PB + k] = jnp.where(own, q, 0.0)

    wr_cp.wait()
    gw_cp.wait()
    wr = small_buf[0].astype(f32)
    gw = small_buf[1].astype(f32)
    r_acc = jnp.zeros((1, _LN), f32)
    g_acc = jnp.zeros((1, _LN), f32)
    for t in range(DB):
        xt = xf[:, t * _LN:(t + 1) * _LN]
        r_acc = r_acc + xt * wr[t:t + 1, :]
        g_acc = g_acc + xt * gw[t:t + 1, :]
    r_sel = jax.nn.sigmoid(jnp.sum(r_acc, axis=-1, keepdims=True))
    gate = jax.nn.sigmoid(jnp.sum(g_acc, axis=-1, keepdims=True))

    def wq_wait(pair):
        wait_all(wq_buf.at[pl.ds(pair * PB, PB)], sem_wq.at[pair])

    wq_wait(0)
    for k in range(PB):
        q_job(0, k)

    def x1_slot(n, m, job=None):
        wait_all(ring.at[n], sem_ring.at[n])
        q = jnp.concatenate([q_buf[k] for k in range(PB)], axis=1).astype(bf16)
        c = 2 * (n - XS)
        s0 = jnp.dot(q, ring[c], preferred_element_type=f32)
        s1 = jnp.dot(q, ring[c + 1], preferred_element_type=f32)
        if job is not None:
            job()

        @pl.when(n < N_X)
        def _():
            early_start(n)

        @pl.when(n >= N_X)
        def _():
            wq_start(n)
        kv_start(k_hbm, n + D1)
        s_buf[c] = s0
        s_buf[c + 1] = s1
        return jnp.maximum(m, jnp.maximum(s0, s1))

    def row_max(m):
        return jnp.broadcast_to(jnp.max(m, axis=-1, keepdims=True), (8, _LN))

    with scope("x1"):
        m = jnp.full((8, _LN), -jnp.inf, f32)
        m = jax.lax.fori_loop(XS, NC - PB, x1_slot, m)
        wq_wait(1)
        m = jax.lax.fori_loop(NC - PB, NC,
                              lambda n, m: x1_slot(n, m, lambda: q_job(1, n - (NC - PB))), m)
        m_buf[0] = row_max(m)

    def k_slot(p, c, m, job=None):
        n = p * NC + c
        wait_all(ring.at[c], sem_ring.at[c])
        q = jnp.concatenate([q_buf[p * PB + k] for k in range(PB)], axis=1).astype(bf16)
        s = jnp.dot(q, ring[c], preferred_element_type=f32)
        if job is not None:
            job()
        k_phase_start(n)
        s_buf[n] = s
        return jnp.maximum(m, s)

    def ffn_job(j):
        col = mo(srl(j, 1) * _LN, _LN)
        h_buf[j] = jnp.dot(x8_buf[...].astype(bf16),
                           wgu_buf[jnp.bitwise_and(j, 1), :, pl.ds(col, _LN)],
                           preferred_element_type=f32)

    FP = _NP - 2
    assert S_D1 + 6 <= FP * NC + (NC - PB - FB)

    def k_period(p, carry):
        with scope("kper"):
            nq = jnp.where(p < _NP - 1, PB, 0)
            nf = jnp.where(p >= FP, FB, 0)
            m = jnp.full((8, _LN), -jnp.inf, f32)
            m = jax.lax.fori_loop(0, NC - nq - nf, lambda c, m: k_slot(p, c, m), m)

            @pl.when(p == FP)
            def _():
                wait_all(wgu_buf, sem_gu.at[0])
            jb = (p - FP) * FB - (NC - nq - nf)
            m = jax.lax.fori_loop(NC - nq - nf, NC - nq,
                                  lambda c, m: k_slot(p, c, m, lambda: ffn_job(jb + c)), m)

            @pl.when(p < _NP - 1)
            def _():
                wq_wait(p + 1)
            m = jax.lax.fori_loop(
                NC - nq, NC,
                lambda c, m: k_slot(p, c, m, lambda: q_job(p + 1, c - (NC - PB))), m)
            m_buf[p] = row_max(m)
        return carry
    jax.lax.fori_loop(1, _NP, k_period, 0)

    for ch in range(FB):
        h_buf[2 * ch] = jax.nn.silu(h_buf[2 * ch]) * h_buf[2 * ch + 1]

    def prob(n):
        return jnp.exp((s_buf[n] - m_buf[srl(n, 5)]) * scale)

    def pv_part(e, c):
        eb = e.astype(bf16)
        return [jax.lax.dot_general(eb, ring[c, pl.ds(k * VR, VR), :], (((1,), (1,)), ((), ())),
                                    preferred_element_type=f32) for k in range(VS)]

    def v_slot(p, c, st, job=None):
        e, l, o = st
        n = p * NC + c
        wait_all(ring.at[c], sem_ring.at[c])
        pv = pv_part(e, c)
        if job is not None:
            job()
        v_phase_start(n)
        l = l + e
        e = prob(n + 1)
        return e, l, tuple(a + b for a, b in zip(o, pv))

    def o_part(ob, pair, col):
        acc = None
        for k in range(VS):
            row = pair * _PR + k * VR
            if not isinstance(row, int):
                row = mo(row, VR)
            t = jnp.dot(ob[k], wo_buf[pl.ds(row, VR), pl.ds(col, _LN)],
                        preferred_element_type=f32)
            acc = t if acc is None else acc + t
        return acc

    def inv_sum(l):
        return 1.0 / jnp.sum(l, axis=-1, keepdims=True)

    def o_job(pair, cb):
        ob = [ob_buf[k].astype(bf16) for k in range(VS)]
        a_buf[cb] += o_part(ob, pair, mo(cb * _LN, _LN)) * inv_sum(l_buf[...])

    def d_job(ch):
        y_buf[...] += jnp.dot(h_buf[2 * ch].astype(bf16),
                              wd_buf[pl.ds(mo(ch * _LN, _LN), _LN), :],
                              preferred_element_type=f32)

    def own_rows(o):
        rr = jax.lax.broadcasted_iota(jnp.int32, (8, VR), 0)
        return [jnp.where(rr == (k * VR) // _DH, o[k], 0.0) for k in range(VS)]

    DP = 6
    assert DP + WD_A <= _NP - 1 and OC >= 8

    def v_period(p, st):
        with scope("vper"):
            e, l, o = st
            no = jnp.where(p >= 1, DB, 0)
            last = p == _NP - 1
            nd = jnp.where(last, WD_B - WD_A,
                           jnp.where(jnp.logical_and(p >= DP, p < DP + WD_A), 1, 0))
            db = jnp.where(last, WD_A, p - DP) - (OC + no)
            ob = own_rows(o)
            for k in range(VS):
                ob_buf[k] = ob[k]
            l_buf[...] = l
            st = (e, jnp.zeros((8, _LN), f32), tuple(jnp.zeros((8, VR), f32) for _ in range(VS)))
            st = jax.lax.fori_loop(0, OC, lambda c, st: v_slot(p, c, st), st)

            @pl.when(p >= 1)
            def _():
                wait_all(wo_buf.at[pl.ds(mo((p - 1) * _PR, _PR), _PR)], sem_wo.at[p - 1])
            st = jax.lax.fori_loop(
                OC, OC + no, lambda c, st: v_slot(p, c, st, lambda: o_job(p - 1, c - OC)), st)

            @pl.when(p == DP)
            def _():
                wait_all(wd_buf.at[pl.ds(0, WD_A * _LN)], sem_wd.at[0])

            @pl.when(last)
            def _():
                wait_all(wd_buf.at[pl.ds(WD_A * _LN, (WD_B - WD_A) * _LN)], sem_wd.at[1])
            st = jax.lax.fori_loop(OC + no, OC + no + nd,
                                   lambda c, st: v_slot(p, c, st, lambda: d_job(db + c)), st)
            st = jax.lax.fori_loop(OC + no + nd, NC - last.astype(jnp.int32),
                                   lambda c, st: v_slot(p, c, st), st)
        return st
    st0 = (prob(0), jnp.ones((8, _LN), f32), tuple(jnp.zeros((8, VR), f32) for _ in range(VS)))
    e, l, o = jax.lax.fori_loop(0, _NP, v_period, st0)

    with scope("tail"):
        wait_all(wo_buf.at[pl.ds((_NP - 1) * _PR, _PR)], sem_wo.at[_NP - 1])
        inv = inv_sum(l + e)
        cy = (1.0 - gate) * r_sel
        res = (1.0 - gate) * (xf + xf * 0.0) + cy * y_buf[0:1, :]
        res = [res[:, cb * _LN:(cb + 1) * _LN] for cb in range(DB)]
        wait_all(ring.at[NC - 1], sem_ring.at[NC - 1])
        pv = pv_part(e, NC - 1)
        ob = [t.astype(bf16) for t in own_rows([a + b for a, b in zip(o, pv)])]
        for cb in range(DB):
            a = a_buf[cb] + o_part(ob, _NP - 1, cb * _LN) * inv
            res[cb] = res[cb] + gate * (a[0:1, :] + a[1:2, :])
        i = 0
        for g in TAILG:
            for j in range(i, i + g):
                tail_copy(j).wait()
            for j in range(i, i + g):
                ch, c0, cn = tail_parts[j]
                y = jnp.dot(h_buf[2 * ch].astype(bf16),
                            wd_buf[pl.ds(ch * _LN, _LN), pl.ds(c0 * _LN, cn * _LN)],
                            preferred_element_type=f32)
                for cb in range(cn):
                    res[c0 + cb] = res[c0 + cb] + cy * y[0:1, cb * _LN:(cb + 1) * _LN]
            i += g
        assert i == len(tail_parts)
        o_ref[...] = jnp.concatenate(res, axis=1).astype(o_ref.dtype)


def _build(D1=16, SCOPES=False, TAILP=((10, 0, 5), (11, 0, 1), (11, 1, 4)), TAILG=(2, 1), OC=8):
    def fn(A_x, A_k_cache, A_v_cache, A_wq, A_wo, B_x, B_w_r, B_w_gate, B_w_up, B_w_down, gate_w):
        B, Sq, D = A_x.shape
        _, Hkv, SK, Dh = A_k_cache.shape
        assert B == 1 and Sq == 1 and Hkv == _HQ and Dh == _DH
        W = min(4096, max(256, SK // 4))
        F = B_w_gate.shape[1]
        n_rows = _HQ * _DH
        NC = W // _LN
        DB, FB, PB = D // _LN, F // _LN, _PR // _LN
        bf16, f32 = jnp.bfloat16, jnp.float32

        x = A_x.reshape(1, D)
        kt = jnp.swapaxes(A_k_cache, 2, 3).reshape(n_rows, SK)
        vt = jnp.swapaxes(A_v_cache, 2, 3).reshape(n_rows, SK)
        wr = B_w_r.reshape(DB, _LN)
        gw = gate_w.reshape(DB, _LN)

        any_spec = pl.BlockSpec(memory_space=pl.ANY)
        out = pl.pallas_call(
            functools.partial(_kernel, D1=D1, W=W, SK=SK, D=D, F=F, SCOPES=SCOPES, TAILP=TAILP, TAILG=TAILG, OC=OC),
            in_specs=[any_spec] * 10,
            out_specs=pl.BlockSpec(memory_space=pltpu.VMEM),
            out_shape=jax.ShapeDtypeStruct((1, D), bf16),
            scratch_shapes=[
                pltpu.VMEM((1, D), bf16),
                pltpu.VMEM((2, DB, _LN), bf16),
                pltpu.VMEM((_NP * PB, D, _LN), bf16),
                pltpu.VMEM((2, D, F), bf16),
                pltpu.VMEM((n_rows, D), bf16),
                pltpu.VMEM((F, D), bf16),
                pltpu.VMEM((NC, _PR, _LN), bf16),
                pltpu.VMEM((8, D), f32),
                pltpu.VMEM((_NP * PB, 8, _LN), f32),
                pltpu.VMEM((_NP * NC, 8, _LN), f32),
                pltpu.VMEM((_NP, 8, _LN), f32),
                pltpu.VMEM((4, 8, _PR // 4), f32),
                pltpu.VMEM((8, _LN), f32),
                pltpu.VMEM((2 * FB, 8, _LN), f32),
                pltpu.VMEM((DB, 8, _LN), f32),
                pltpu.VMEM((8, D), f32),
                pltpu.SemaphoreType.DMA((3,)),
                pltpu.SemaphoreType.DMA((_NP,)),
                pltpu.SemaphoreType.DMA((1,)),
                pltpu.SemaphoreType.DMA((_NP,)),
                pltpu.SemaphoreType.DMA((2 + len(TAILP),)),
                pltpu.SemaphoreType.DMA((NC,)),
            ],
            compiler_params=_compiler_params(vmem_limit_bytes=100 * 1024 * 1024,
                                             disable_bounds_checks=True,
                                             disable_semaphore_checks=True),
        )(x, kt, vt, A_wq, A_wo, wr, B_w_gate, B_w_up, B_w_down, gw)
        return out.reshape(B, Sq, D)
    return fn


@jax.jit
def pallas_gated_mix__sliding_block_cached__moe_arch_mod__decode_kernel(
    A_x: jax.Array,
    A_k_cache: jax.Array,
    A_v_cache: jax.Array,
    A_wq: jax.Array,
    A_wo: jax.Array,
    B_x: jax.Array,
    B_w_r: jax.Array,
    B_w_gate: jax.Array,
    B_w_up: jax.Array,
    B_w_down: jax.Array,
    gate_w: jax.Array,
):
    return _build()(A_x, A_k_cache, A_v_cache, A_wq, A_wo, B_x, B_w_r,
                    B_w_gate, B_w_up, B_w_down, gate_w)
```

```python
import dataclasses
import functools

import jax
import jax.numpy as jnp
import jax.experimental.pallas as pl
import jax.experimental.pallas.tpu as pltpu

_HQ = 32
_DH = 192
_LN = 128


def _const_div(n, d, hi):
    for sh in range(1, 20):
        m = -(-(1 << sh) // d)
        if all((v * m) >> sh == v // d for v in range(hi)):
            return jax.lax.shift_right_logical(n * m, sh)
    raise ValueError("no multiplier")


def _compiler_params(**kw):
    names = {f.name for f in dataclasses.fields(pltpu.CompilerParams)}
    return pltpu.CompilerParams(**{k: v for k, v in kw.items() if k in names})


class _NoScope:
    def __enter__(self):
        return self

    def __exit__(self, *a):
        return False


def _kernel(x_hbm, k_hbm, v_hbm, wq_hbm, wo_hbm, wr_hbm, wg_hbm, wu_hbm, wd_hbm, gw_hbm,
            o_ref,
            x_buf, small_buf, wq_buf, wgu_buf, wo_buf, wd_buf, ring,
            x8_buf, q_buf, qh_buf, s_buf, m_buf, acc_buf, l_buf, h_buf, a_buf, y_buf,
            sem_small, sem_wq, sem_gu, sem_wo, sem_wd, sem_ring,
            *, D1, W, SK, D, F, SCOPES, TAILP, TAILG, OC, MG, RA, CS, FIRST):
    f32, bf16 = jnp.float32, jnp.bfloat16
    scope = jax.named_scope if SCOPES else (lambda name: _NoScope())
    NC = W // _LN
    NS = _HQ * NC
    NH = NS // 2
    DB = D // _LN
    FB = F // _LN
    QB = _HQ * _DH // _LN
    RT = _DH // 8
    col0 = SK - W
    assert NC == 32 and D1 == NC // 2 and D % _LN == 0 and F % _LN == 0 and DB % 2 == 1
    QC = 8 * _LN
    QS = QB * _LN // QC
    QK = (_LN // 8) * QS
    S_WG = DB * QK
    GC = 6 * _LN
    N_WG = (D // 8) * (F // GC)
    UC = 4 * _LN
    UB = F // UC
    N_WU = (D // 8) * UB
    S_WU = S_WG + N_WG
    S_D1 = S_WU + N_WU
    N_D1 = NS - S_D1
    WD_B = N_D1 * 8 // _LN
    PU = 16
    OU = _DH * DB // PU
    assert N_D1 * 8 == WD_B * _LN and 2 * CS + (NC - CS) == OU
    HB = NC // 2
    assert (S_WU - NH) % HB == 0 and (S_D1 - NH) % HB == 0
    JB = 6
    JN = QB // JB
    assert F // GC == 2 and S_WG + MG + 3 * JN == NH
    scale = _DH ** -0.5

    mo = pl.multiple_of
    srl = jax.lax.shift_right_logical

    def kv_start(src, t, slot):
        row = mo(srl(t, 5) * _DH, _DH // 3)
        c = jnp.bitwise_and(t, NC - 1)
        col = mo(col0 + c * _LN, _LN)
        pltpu.make_async_copy(src.at[pl.ds(row, _DH), pl.ds(col, _LN)],
                              ring.at[slot], sem_ring.at[c]).start(priority=1)

    def wait_all(ref, sem):
        pltpu.make_async_copy(ref, ref, sem).wait()

    def wd_start(n):
        sl = pl.ds(mo((n - S_D1) * 8, 8), 8)
        pltpu.make_async_copy(wd_hbm.at[sl], wd_buf.at[sl], sem_wd.at[0]).start(priority=0)

    def wq_start(n):
        band = _const_div(n, QS, NS)
        sl = (pl.ds(mo(band * 8, 8), 8), pl.ds(mo((n - band * QS) * QC, QC), QC))
        pltpu.make_async_copy(wq_hbm.at[sl], wq_buf.at[sl],
                              sem_wq.at[_const_div(n, QK, NS)]).start(priority=0)

    def wg_start(n):
        u = n - S_WG
        sl = (pl.ds(mo(srl(u, 1) * 8, 8), 8), pl.ds(mo(jnp.bitwise_and(u, 1) * GC, _LN), GC))
        pltpu.make_async_copy(wg_hbm.at[sl], wgu_buf.at[0].at[sl], sem_gu.at[0]).start(priority=0)

    def wu_start(n):
        u = n - S_WU
        r = _const_div(u, UB, NS)
        sl = (pl.ds(mo(r * 8, 8), 8), pl.ds(mo((u - r * UB) * UC, _LN), UC))
        pltpu.make_async_copy(wu_hbm.at[sl], wgu_buf.at[1].at[sl], sem_gu.at[0]).start(priority=0)

    def b_q1(t):
        @pl.when(t < NS)
        def _():
            kv_start(k_hbm, t, t)

        @pl.when(t >= NS)
        def _():
            kv_start(v_hbm, t - NS, t - NS)

    tail_parts = TAILP

    def tail_copy(i):
        ch, c0, cn = tail_parts[i]
        sl = (pl.ds(ch * _LN, _LN), pl.ds(c0 * _LN, cn * _LN))
        return pltpu.make_async_copy(wd_hbm.at[sl], wd_buf.at[sl], sem_wd.at[1 + i])

    def v_phase_start(n, pos, un):
        @pl.when(pos < _HQ * OU)
        def _():
            sl = pl.ds(mo(pos * PU, PU), un * PU)
            pltpu.make_async_copy(wo_hbm.at[sl], wo_buf.at[sl],
                                  sem_wo.at[_const_div(pos, OU, 2 * NS + 8)]).start(priority=0)
        t = n + D1

        @pl.when(t < NS)
        def _():
            kv_start(v_hbm, t, jnp.bitwise_and(t, NC - 1))

    x_cp = pltpu.make_async_copy(x_hbm, x_buf, sem_small.at[0])
    wr_cp = pltpu.make_async_copy(wr_hbm, small_buf.at[0], sem_small.at[1])
    gw_cp = pltpu.make_async_copy(gw_hbm, small_buf.at[1], sem_small.at[2])
    for j in range(D1):
        pltpu.make_async_copy(k_hbm.at[pl.ds(0, _DH), pl.ds(col0 + j * _LN, _LN)],
                              ring.at[j], sem_ring.at[j]).start(priority=1)
    x_cp.start(priority=0)
    wr_cp.start(priority=0)
    gw_cp.start(priority=0)
    a_buf[...] = jnp.zeros(a_buf.shape, f32)
    y_buf[...] = jnp.zeros(y_buf.shape, f32)
    q_buf[...] = jnp.zeros(q_buf.shape, f32)
    h_buf[...] = jnp.zeros(h_buf.shape, f32)

    lane_id = jax.lax.broadcasted_iota(jnp.int32, (8, _LN), 1)

    def k_wait(n):
        wait_all(ring.at[n], sem_ring.at[jnp.bitwise_and(n, NC - 1)])

    def a_slot(n, job=None, q0=wq_start):
        k_wait(n)
        fin = job() if job is not None else None
        q0(n)
        kv_start(k_hbm, n + D1, n + D1)
        if fin is not None:
            fin()

    def loop(lo, hi, body):
        def b(n, c):
            body(n)
            return c
        jax.lax.fori_loop(lo, hi, b, 0)

    NPREP = 2 * D1
    with scope("a0"):
        loop(0, NPREP, a_slot)

    a_slot(jnp.int32(NPREP))
    x_cp.wait()
    wr_cp.wait()
    gw_cp.wait()
    xf = x_buf[...].astype(f32)
    wr = small_buf[0].astype(f32)
    gw = small_buf[1].astype(f32)
    r_acc = jnp.zeros((8, _LN), f32)
    g_acc = jnp.zeros((8, _LN), f32)
    for t in range(DB):
        xt = jnp.broadcast_to(xf[:, t * _LN:(t + 1) * _LN], (8, _LN))
        x8_buf[t] = xt
        r_acc = r_acc + xt * jnp.broadcast_to(wr[t:t + 1, :], (8, _LN))
        g_acc = g_acc + xt * jnp.broadcast_to(gw[t:t + 1, :], (8, _LN))
    r_sel = jax.nn.sigmoid(jnp.sum(r_acc, axis=-1, keepdims=True))
    gate = jax.nn.sigmoid(jnp.sum(g_acc, axis=-1, keepdims=True))

    def q_job(ch, g):
        last = isinstance(ch, int)
        row = ch * _LN if last else mo(ch * _LN, _LN)
        t = jnp.dot(x8_buf[ch].astype(bf16),
                    wq_buf[pl.ds(row, _LN), pl.ds(mo(g * (JB * _LN), _LN), JB * _LN)],
                    preferred_element_type=f32)

        def fin():
            q = [q_buf[g * JB + i] + t[:, i * _LN:(i + 1) * _LN] for i in range(JB)]
            if not last:
                for i in range(JB):
                    q_buf[g * JB + i] = q[i]
                return
            for i in range(JB // 3):
                b0, b1, b2 = q[3 * i:3 * i + 3]
                k = g * (4 * JB // 3) + 4 * i
                qh_buf[k] = b0
                qh_buf[k + 1] = jnp.where(lane_id < 32, pltpu.roll(b0, 32, 1), pltpu.roll(b1, 32, 1))
                qh_buf[k + 2] = jnp.where(lane_id < 64, pltpu.roll(b1, 64, 1), pltpu.roll(b2, 64, 1))
                qh_buf[k + 3] = pltpu.roll(b2, 96, 1)
        return fin

    def wq_wait(ch):
        row = ch * _LN if isinstance(ch, int) else mo(ch * _LN, _LN)
        wait_all(wq_buf.at[pl.ds(row, _LN)], sem_wq.at[ch])

    def a_late(n):
        @pl.when(n < S_WG)
        def _():
            wq_start(n)

        @pl.when(n >= S_WG)
        def _():
            wg_start(n)

    def q_jobs(ch, n0, q0):
        def three(g):
            n = n0 + 3 * g
            a_slot(n, lambda: q_job(ch, g), q0)
            a_slot(n + 1, None, q0)
            a_slot(n + 2, None, q0)
        loop(0, JN, three)

    with scope("a1"):
        loop(NPREP + 1, QK + MG, a_slot)

        def a_chunk(ch):
            wq_wait(ch)
            n0 = (ch + 1) * QK + MG
            q_jobs(ch, n0, wq_start)
            loop(n0 + 3 * JN, n0 + QK, lambda n: a_slot(n, None, a_late))
        loop(0, DB - 1, a_chunk)
        wq_wait(DB - 1)
        q_jobs(DB - 1, S_WG + MG, wg_start)

    def lane_max(m):
        return jnp.broadcast_to(jnp.max(m, axis=-1, keepdims=True), (8, _LN))

    KR = _DH // 2

    def b_slot(q0, h, i, m, job=None):
        n = NH + h * HB + 2 * i
        t = h * NC + 4 * i
        k_wait(n)
        q0(n)
        k_wait(n + 1)
        q = [qh_buf[2 * h + k][:, :KR].astype(bf16) for k in range(2)]
        s = [jnp.dot(q[0], ring[t + j, pl.ds(0, KR), :], preferred_element_type=f32)
             + jnp.dot(q[1], ring[t + j, pl.ds(KR, KR), :], preferred_element_type=f32)
             for j in range(4)]
        if job is not None:
            job()
        q0(n + 1)
        b_q1(n + D1)
        b_q1(n + 1 + D1)
        for j in range(4):
            s_buf[t + j] = s[j]
        return jnp.maximum(jnp.maximum(m, jnp.maximum(s[0], s[1])), jnp.maximum(s[2], s[3]))

    m_init = jnp.full((8, _LN), -jnp.inf, f32)

    def b_period(q0, h, m_prev):
        with scope("bper"):
            def job():
                m_buf[jnp.maximum(h - 1, 0)] = lane_max(m_prev)
            m = b_slot(q0, h, 0, m_init, job)
            m = jax.lax.fori_loop(1, NC // 4, lambda i, m: b_slot(q0, h, i, m), m)
        return m
    h1, h2 = (S_WU - NH) // HB, (S_D1 - NH) // HB
    m_last = jax.lax.fori_loop(0, h1, functools.partial(b_period, wg_start), m_init)
    m_last = jax.lax.fori_loop(h1, h2, functools.partial(b_period, wu_start), m_last)
    m_last = jax.lax.fori_loop(h2, _HQ, functools.partial(b_period, wd_start), m_last)
    m_buf[_HQ - 1] = lane_max(m_last)

    def prob(n):
        return jnp.exp((s_buf[n] - m_buf[srl(n, 5)]) * scale)

    def pv_add(acc, e, c):
        return acc + ring[c].astype(f32).reshape(RT, 8, _LN) * e[None]

    def v_slot(h, c, st, job=None, un=2):
        pos, e, l, acc = st
        n = h * NC + c
        wait_all(ring.at[c], sem_ring.at[c])
        if FIRST:
            v_phase_start(n, pos, un)
        acc = pv_add(acc, e, c)
        if job is not None:
            job()
        if not FIRST:
            v_phase_start(n, pos, un)
        return pos + un, prob(n + 1), l + e, acc

    def lane_sum(v):
        return jnp.broadcast_to(jnp.sum(v, axis=-1, keepdims=True), v.shape)

    def fin_job():
        acc_buf[...] = lane_sum(acc_buf[...])
        l_buf[...] = 1.0 / lane_sum(l_buf[...])

    def o_tiles(col, row, nt):
        w = wo_buf[pl.ds(row, nt * DB * 8), :].astype(f32).reshape(nt, DB, 8, _LN)
        return jnp.sum(w * col[:, None], axis=0)

    OJ = 4
    OT = RT // OJ

    def o_job(h, k):
        col = acc_buf[pl.ds(k * OT, OT)]
        a_buf[...] += o_tiles(col, mo((h * OJ + k) * (OT * DB * 8), 16), OT) * l_buf[...][None]

    def f_job(j):
        ch = srl(j, 1)
        up = jnp.bitwise_and(j, 1)
        x8 = jnp.concatenate([x8_buf[t] for t in range(DB)], axis=1).astype(bf16)
        t = jnp.dot(x8, wgu_buf[up, :, pl.ds(mo(ch * _LN, _LN), _LN)], preferred_element_type=f32)
        h_buf[ch] = jnp.where(up == 1, jax.nn.silu(h_buf[ch]), 1.0) * t

    def d_job(ch):
        y = jnp.dot(h_buf[ch].astype(bf16), wd_buf[pl.ds(mo(ch * _LN, _LN), _LN), :],
                    preferred_element_type=f32)
        for cb in range(DB):
            y_buf[cb] += y[:, cb * _LN:(cb + 1) * _LN]

    DP = FB + 1
    assert DP + WD_B < _HQ and OC + 1 + OJ + 2 <= NC - D1 <= CS

    def v_period(h, st):
        with scope("vper"):
            pos, e, l, acc = st
            first = (h >= 1).astype(jnp.int32)
            last = h == _HQ - 1
            nf = jnp.where(h < FB, 2, 0)
            nd = jnp.logical_and(h >= DP, h < DP + WD_B).astype(jnp.int32)
            acc_buf[...] = acc
            l_buf[...] = l
            st = (pos, e, jnp.zeros((8, _LN), f32), jnp.zeros((RT, 8, _LN), f32))
            st = jax.lax.fori_loop(0, OC, lambda c, st: v_slot(h, c, st), st)
            st = v_slot(h, jnp.int32(OC), st, fin_job)

            @pl.when(h >= 1)
            def _():
                wait_all(wo_buf.at[pl.ds(mo((h - 1) * (_DH * DB), 64), _DH * DB)], sem_wo.at[h - 1])
            c1 = OC + 1 + first * OJ
            st = jax.lax.fori_loop(
                OC + 1, c1, lambda c, st: v_slot(h, c, st, lambda: o_job(h - 1, c - OC - 1)), st)

            @pl.when(h == 0)
            def _():
                wait_all(wgu_buf, sem_gu.at[0])
            c2 = c1 + nf
            st = jax.lax.fori_loop(
                c1, c2, lambda c, st: v_slot(h, c, st, lambda: f_job(2 * h + c - c1)), st)

            @pl.when(h == DP)
            def _():
                wait_all(wd_buf.at[pl.ds(0, WD_B * _LN)], sem_wd.at[0])
            c3 = c2 + nd
            st = jax.lax.fori_loop(c2, c3, lambda c, st: v_slot(h, c, st, lambda: d_job(h - DP)), st)
            st = jax.lax.fori_loop(c3, NC - D1, lambda c, st: v_slot(h, c, st), st)

            @pl.when(last)
            def _():
                for i in range(len(tail_parts)):
                    tail_copy(i).start(priority=1)
            cs = jnp.where(h < RA, NC, CS)
            st = jax.lax.fori_loop(NC - D1, cs, lambda c, st: v_slot(h, c, st), st)
            st = jax.lax.fori_loop(cs, NC - last.astype(jnp.int32),
                                   lambda c, st: v_slot(h, c, st, un=1), st)
        return st
    st0 = (jnp.int32(0), prob(0), jnp.ones((8, _LN), f32), jnp.zeros((RT, 8, _LN), f32))
    _, e, l, acc = jax.lax.fori_loop(0, _HQ, v_period, st0)

    with scope("tail"):
        wait_all(wo_buf.at[pl.ds((_HQ - 1) * _DH * DB, _DH * DB)], sem_wo.at[_HQ - 1])
        inv = 1.0 / lane_sum(l + e)
        cy = (1.0 - gate) * r_sel
        res = []
        for cb in range(DB):
            xt = x8_buf[cb]
            res.append(((1.0 - gate) * (xt + xt * 0.0) + cy * y_buf[cb])[0:1])
        wait_all(ring.at[NC - 1], sem_ring.at[NC - 1])
        col = lane_sum(pv_add(acc, e, NC - 1))
        a = a_buf[...] + o_tiles(col, (_HQ - 1) * _DH * DB, RT) * inv[None]
        for cb in range(DB):
            res[cb] = res[cb] + gate[0:1] * jnp.sum(a[cb], axis=0, keepdims=True)
        cy = cy[0:1]
        i = 0
        for g in TAILG:
            for j in range(i, i + g):
                tail_copy(j).wait()
            for j in range(i, i + g):
                ch, c0, cn = tail_parts[j]
                y = jnp.dot(h_buf[ch].astype(bf16),
                            wd_buf[pl.ds(ch * _LN, _LN), pl.ds(c0 * _LN, cn * _LN)],
                            preferred_element_type=f32)
                for cb in range(cn):
                    res[c0 + cb] = res[c0 + cb] + cy * y[0:1, cb * _LN:(cb + 1) * _LN]
            i += g
        assert i == len(tail_parts)
        o_ref[...] = jnp.concatenate(res, axis=1).astype(o_ref.dtype)


def _build(D1=16, SCOPES=False, TAILP=((9, 0, 5), (10, 0, 5), (11, 0, 1), (11, 1, 4)),
           TAILG=(3, 1), OC=8, MG=8, RA=3, CS=28, FIRST=True):
    def fn(A_x, A_k_cache, A_v_cache, A_wq, A_wo, B_x, B_w_r, B_w_gate, B_w_up, B_w_down, gate_w):
        B, Sq, D = A_x.shape
        _, Hkv, SK, Dh = A_k_cache.shape
        assert B == 1 and Sq == 1 and Hkv == _HQ and Dh == _DH
        W = min(4096, max(256, SK // 4))
        F = B_w_gate.shape[1]
        n_rows = _HQ * _DH
        NC = W // _LN
        DB, FB = D // _LN, F // _LN
        bf16, f32 = jnp.bfloat16, jnp.float32

        def tiles(w):
            r = w.shape[0]
            return w.reshape(r // 8, 8, DB, _LN).transpose(0, 2, 1, 3).reshape(r * DB, _LN)

        x = A_x.reshape(1, D)
        kt = jnp.swapaxes(A_k_cache, 2, 3).reshape(n_rows, SK)
        vt = jnp.swapaxes(A_v_cache, 2, 3).reshape(n_rows, SK)
        wr = B_w_r.reshape(DB, _LN)
        gw = gate_w.reshape(DB, _LN)

        any_spec = pl.BlockSpec(memory_space=pl.ANY)
        out = pl.pallas_call(
            functools.partial(_kernel, D1=D1, W=W, SK=SK, D=D, F=F, SCOPES=SCOPES, TAILP=TAILP,
                              TAILG=TAILG, OC=OC, MG=MG, RA=RA, CS=CS, FIRST=FIRST),
            in_specs=[any_spec] * 10,
            out_specs=pl.BlockSpec(memory_space=pltpu.VMEM),
            out_shape=jax.ShapeDtypeStruct((1, D), bf16),
            scratch_shapes=[
                pltpu.VMEM((1, D), bf16),
                pltpu.VMEM((2, DB, _LN), bf16),
                pltpu.VMEM((D, n_rows), bf16),
                pltpu.VMEM((2, D, F), bf16),
                pltpu.VMEM((n_rows * DB, _LN), bf16),
                pltpu.VMEM((F, D), bf16),
                pltpu.VMEM((_HQ * NC, _DH, _LN), bf16),
                pltpu.VMEM((DB, 8, _LN), f32),
                pltpu.VMEM((n_rows // _LN, 8, _LN), f32),
                pltpu.VMEM((2 * _HQ, 8, _LN), f32),
                pltpu.VMEM((_HQ * NC, 8, _LN), f32),
                pltpu.VMEM((_HQ, 8, _LN), f32),
                pltpu.VMEM((_DH // 8, 8, _LN), f32),
                pltpu.VMEM((8, _LN), f32),
                pltpu.VMEM((FB, 8, _LN), f32),
                pltpu.VMEM((DB, 8, _LN), f32),
                pltpu.VMEM((DB, 8, _LN), f32),
                pltpu.SemaphoreType.DMA((3,)),
                pltpu.SemaphoreType.DMA((DB,)),
                pltpu.SemaphoreType.DMA((1,)),
                pltpu.SemaphoreType.DMA((_HQ,)),
                pltpu.SemaphoreType.DMA((1 + len(TAILP),)),
                pltpu.SemaphoreType.DMA((NC,)),
            ],
            compiler_params=_compiler_params(vmem_limit_bytes=100 * 1024 * 1024,
                                             disable_bounds_checks=True,
                                             disable_semaphore_checks=True),
        )(x, kt, vt, A_wq, tiles(A_wo), wr, B_w_gate, B_w_up, B_w_down, gw)
        return out.reshape(B, Sq, D)
    return fn


@jax.jit
def pallas_gated_mix__sliding_block_cached__moe_arch_mod__decode_kernel(
    A_x: jax.Array,
    A_k_cache: jax.Array,
    A_v_cache: jax.Array,
    A_wq: jax.Array,
    A_wo: jax.Array,
    B_x: jax.Array,
    B_w_r: jax.Array,
    B_w_gate: jax.Array,
    B_w_up: jax.Array,
    B_w_down: jax.Array,
    gate_w: jax.Array,
):
    return _build()(A_x, A_k_cache, A_v_cache, A_wq, A_wo, B_x, B_w_r,
                    B_w_gate, B_w_up, B_w_down, gate_w)
```

```python
import dataclasses
import functools
import math

import jax
import jax.numpy as jnp
import jax.experimental.pallas as pl
import jax.experimental.pallas.tpu as pltpu

_HQ = 32
_DH = 192
_LN = 128


def _const_div(n, d, hi):
    if isinstance(n, int):
        return n // d
    for sh in range(1, 20):
        m = -(-(1 << sh) // d)
        if all((v * m) >> sh == v // d for v in range(hi)):
            return jax.lax.shift_right_logical(n * m, sh)
    raise ValueError("no multiplier")


def _compiler_params(**kw):
    names = {f.name for f in dataclasses.fields(pltpu.CompilerParams)}
    return pltpu.CompilerParams(**{k: v for k, v in kw.items() if k in names})


class _NoScope:
    def __enter__(self):
        return self

    def __exit__(self, *a):
        return False


def _kernel(x_hbm, k_hbm, v_hbm, wq_hbm, wo_hbm, wr_hbm, wg_hbm, wu_hbm, wd_hbm, gw_hbm,
            o_ref,
            x_buf, small_buf, wq_buf, wgu_buf, wo_buf, wd_buf, ring,
            x8_buf, xc_buf, g_buf, q_buf, qc_buf, s_buf, m_buf, acc_buf, l_buf, h_buf, hc_buf,
            a_buf,
            sem_small, sem_gu, sem_wo, sem_wd, sem_ring,
            *, D1, W, SK, D, F, ST, SCOPES, TQ0, TQA, TAILP, ORDER, SPLIT, OC, JC):
    f32, bf16 = jnp.float32, jnp.bfloat16
    scope = jax.named_scope if SCOPES else (lambda name: _NoScope())
    NC = W // _LN
    NS = _HQ * NC
    DB = D // _LN
    FB = F // _LN
    QB = _HQ * _DH // _LN
    RT = _DH // 8
    BT = _LN // 8
    col0 = SK - W
    assert NC == 32 and D1 == NC // 2 and D % _LN == 0 and F % _LN == 0
    WB = (D // 8) * QB // ST
    WC = 2 * _LN
    NW = ST // 2
    WR = QB // math.gcd(ST, QB)
    WK = WR * ST // QB
    assert WB * ST == (D // 8) * QB and WB % WR == 0 and NW % NC == 0 and QB % 2 == 0
    PT = 3
    GP = FB // PT
    N_WG = (D // 8) * GP
    WD_B = 9
    S_WU = N_WG
    S_WD = 2 * N_WG
    S_WO = S_WD + WD_B * BT * DB // PT
    OP = RT * DB // PT
    S_V = NW + NS
    assert GP == 4 and FB % PT == 0 and (WD_B * BT * DB) % PT == 0 and (RT * DB) % PT == 0
    assert S_WO + _HQ * OP == S_V + NS - D1 and NW < S_WU and S_WO < S_V - D1
    assert S_WU % 2 == 0 and S_WO % 2 == 0
    scale = _DH ** -0.5

    def mo(v, m):
        return v if isinstance(v, int) else pl.multiple_of(v, m)
    srl = jax.lax.shift_right_logical

    def kv_start(src, t):
        row = mo((t >> 5) * _DH, _DH // 3)
        c = t & (NC - 1)
        col = mo(col0 + c * _LN, _LN)
        pltpu.make_async_copy(src.at[pl.ds(row, _DH), pl.ds(col, _LN)],
                              ring.at[c], sem_ring.at[c]).start(priority=1)

    def wq_start(j):
        if not SPLIT:
            pltpu.make_async_copy(wq_hbm.at[:, pl.ds(mo(j * WC, WC), WC)], wq_buf.at[j],
                                  sem_ring.at[j & (NC - 1)]).start(priority=1)
            return
        for i in range(2):
            pltpu.make_async_copy(wq_hbm.at[:, pl.ds(mo(j * WC + i * _LN, _LN), _LN)],
                                  wq_buf.at[j, :, pl.ds(i * _LN, _LN)],
                                  sem_ring.at[j & (NC - 1)]).start(priority=1)

    def wait_all(ref, sem):
        pltpu.make_async_copy(ref, ref, sem).wait()

    def gu_start(src, i, u):
        sl = (pl.ds(mo((u >> 2) * 8, 8), 8), pl.ds(mo((u & 3) * (PT * _LN), _LN), PT * _LN))
        pltpu.make_async_copy(src.at[sl], wgu_buf.at[i].at[sl], sem_gu.at[0]).start(priority=0)

    def wg_start(g):
        gu_start(wg_hbm, 0, g)

    def wu_start(g):
        gu_start(wu_hbm, 1, g - S_WU)

    def wd_start(g):
        sl = pl.ds(mo((g - S_WD) * (PT * 8), 8), PT * 8)
        pltpu.make_async_copy(wd_hbm.at[sl], wd_buf.at[sl], sem_wd.at[0]).start(priority=0)

    def wo_start(g):
        u = g - S_WO
        sl = pl.ds(mo(u * (PT * 8), 8), PT * 8)
        pltpu.make_async_copy(wo_hbm.at[sl], wo_buf.at[sl],
                              sem_wo.at[_const_div(u, OP, _HQ * OP)]).start(priority=0)

    BR = DB * 8
    TB = WD_B * BT

    def band_rows(b0, nb):
        return pl.ds(mo(b0 * BR, 8), nb * BR)

    def tq0_start(i):
        sl = band_rows(TB + i, 1)
        k = int(i >= TQA) if isinstance(i, int) else (i >= TQA).astype(jnp.int32)
        pltpu.make_async_copy(wd_hbm.at[sl], wd_buf.at[sl], sem_wd.at[1 + k]).start(priority=0)

    groups = [(TB, TQA), (TB + TQA, TQ0 - TQA)]
    for nb in TAILP:
        groups.append((sum(groups[-1]), nb))
    assert sum(groups[-1]) == F // 8 and all(b % 2 == 0 and n % 2 == 0 for b, n in groups)
    assert sorted(ORDER) == [i for i, (_, n) in enumerate(groups) if n] and TQ0 <= D1

    x_cp = pltpu.make_async_copy(x_hbm, x_buf, sem_small.at[0])
    wr_cp = pltpu.make_async_copy(wr_hbm, small_buf.at[0], sem_small.at[1])
    gw_cp = pltpu.make_async_copy(gw_hbm, small_buf.at[1], sem_small.at[2])
    wq_start(0)
    x_cp.start(priority=0)
    for j in range(1, D1):
        wq_start(j)
    wr_cp.start(priority=0)
    gw_cp.start(priority=0)
    a_buf[...] = jnp.zeros(a_buf.shape, f32)
    q_buf[...] = jnp.zeros(q_buf.shape, f32)
    h_buf[...] = jnp.zeros(h_buf.shape, f32)

    lane_id = jax.lax.broadcasted_iota(jnp.int32, (8, _LN), 1)
    diag = lane_id - jax.lax.broadcasted_iota(jnp.int32, (8, _LN), 0)

    def lane_sum(v):
        return jnp.broadcast_to(jnp.sum(v, axis=-1, keepdims=True), v.shape)

    def columns(v):
        return lane_sum(jnp.stack([jnp.where(diag == 8 * k, v, 0.0) for k in range(BT)]))

    def loop(lo, hi, body):
        def b(n, c):
            body(n)
            return c
        jax.lax.fori_loop(lo, hi, b, 0)

    def q_add(j):
        w = wq_buf[j].astype(f32)
        for r in range(WR):
            p = r * NW + j
            kb = _const_div(p, QB // 2, WR * NW)
            cb = 2 * p - QB * kb
            xc = [xc_buf[kb + WK * i] for i in range(WB // WR)]
            for jj in range(2):
                acc = q_buf[cb + jj]
                for i in range(WB // WR):
                    b = r + WR * i
                    acc = acc + w[8 * b:8 * b + 8, jj * _LN:(jj + 1) * _LN] * xc[i]
                q_buf[cb + jj] = acc

    def w_slot(j, job, q1=None):
        wait_all(wq_buf.at[j], sem_ring.at[j & (NC - 1)])
        wg_start(j)
        if q1 is None:
            wq_start(j + D1)
        else:
            q1()
        job()

    def x_job(t):
        if t == 0:
            x_cp.wait()
        xt = jnp.broadcast_to(x_buf[:, t * _LN:(t + 1) * _LN].astype(f32), (8, _LN))
        x8_buf[t] = xt
        xc_buf[pl.ds(t * BT, BT)] = columns(xt)

    def gate_job():
        wr_cp.wait()
        gw_cp.wait()
        wr = small_buf[0].astype(f32)
        gw = small_buf[1].astype(f32)
        r_acc = jnp.zeros((8, _LN), f32)
        g_acc = jnp.zeros((8, _LN), f32)
        for t in range(DB):
            xt = x8_buf[t]
            r_acc = r_acc + xt * jnp.broadcast_to(wr[t:t + 1, :], (8, _LN))
            g_acc = g_acc + xt * jnp.broadcast_to(gw[t:t + 1, :], (8, _LN))
        r_sel = jax.nn.sigmoid(lane_sum(r_acc))
        gate = jax.nn.sigmoid(lane_sum(g_acc))
        g_buf[0] = gate
        g_buf[1] = (1.0 - gate) * r_sel

    with scope("w0"):
        for t in range(DB):
            w_slot(t, functools.partial(x_job, t))

        def two(j):
            q_add(j - DB)
            q_add(j)
        loop(DB, 2 * DB, lambda j: w_slot(j, lambda: two(j)))

        def with_gate():
            gate_job()
            q_add(2 * DB)
        w_slot(2 * DB, with_gate)
    with scope("w1"):
        loop(2 * DB + 1, NW - D1, lambda j: w_slot(j, lambda: q_add(j)))
        loop(NW - D1, NW,
             lambda j: w_slot(j, lambda: q_add(j), lambda: kv_start(k_hbm, j + D1 - NW)))

    def row_sum(v):
        return jnp.broadcast_to(jnp.sum(v, axis=0, keepdims=True), (8, _LN))

    def q_fin(h):
        odd = h & 1
        cb = (3 * h) >> 1
        va, vb = row_sum(q_buf[cb]), row_sum(q_buf[cb + 1])
        vm = jnp.where(odd == 1, vb, va)
        lo, hi = diag - 64 * odd, diag + 64 * odd
        t = ([jnp.where(lo == 8 * r, va, 0.0) for r in range(8)]
             + [jnp.where(hi == 8 * r, vm, 0.0) for r in range(8, 16)]
             + [jnp.where(lo == 8 * r, vb, 0.0) for r in range(8)])
        qc_buf[pl.ds(h * RT, RT)] = lane_sum(jnp.stack(t))

    def lane_max(m):
        return jnp.broadcast_to(jnp.max(m, axis=-1, keepdims=True), (8, _LN))

    def score(t):
        p = (ring[t & (NC - 1)].astype(f32).reshape(RT // 4, 4, 8, _LN)
             * qc_buf[pl.ds((t >> 5) * RT, RT)].reshape(RT // 4, 4, 8, _LN))
        p = jnp.sum(p, axis=0)
        s = row_sum((p[0] + p[1]) + (p[2] + p[3]))
        s_buf[t] = s
        return s

    def k_dma(q0, nxt, t):
        c = t & (NC - 1)
        wait_all(ring.at[c], sem_ring.at[c])
        q0(NW + t)
        if nxt:
            kv_start(v_hbm, t + D1 - NS)
        else:
            kv_start(k_hbm, t + D1)

    def k_slot(q0, nxt, t, m):
        c = t & (NC - 1)
        h = srl(t, 5)
        k_dma(q0, nxt, t)
        m = jnp.maximum(jnp.where(c == 0, -jnp.inf, m), score(t))
        m_buf[h] = m

        @pl.when(c == JC)
        def _():
            hp = jnp.maximum(h - 1, 0)
            m_buf[hp] = lane_max(m_buf[hp])
            q_fin(jnp.minimum(h + 1, _HQ - 1))
        return m

    k_dma(wg_start, False, 0)
    q_fin(0)
    k_dma(wg_start, False, 1)
    m = jnp.maximum(score(0), score(1))
    lo = NW + 2
    for hi, q0, nxt in ((S_WU, wg_start, False), (S_WD, wu_start, False), (S_WO, wd_start, False),
                        (S_V - D1, wo_start, False), (S_V, wo_start, True)):
        if nxt:
            e0 = jnp.exp((s_buf[0] - m_buf[0]) * scale)
        with scope("k%d" % lo):
            m = jax.lax.fori_loop(lo - NW, hi - NW, functools.partial(k_slot, q0, nxt), m)
        lo = hi

    def prob(n):
        return jnp.exp((s_buf[n] - m_buf[srl(n, 5)]) * scale)

    def pv_add(acc, e, c):
        return acc + ring[c].astype(f32).reshape(RT, 8, _LN) * e[None]

    def v_slot(h, c, st, job=None, tail=False):
        e, l, acc = st
        n = h * NC + c
        wait_all(ring.at[c], sem_ring.at[c])
        if tail:
            if TQ0 >= D1 - 1:
                tq0_start(c - D1)
            else:
                @pl.when(c - D1 < TQ0)
                def _():
                    tq0_start(c - D1)
        else:
            wo_start(S_V + n)
            kv_start(v_hbm, n + D1)
        acc = pv_add(acc, e, c)
        if job is not None:
            job()
        return prob(n + 1), l + e, acc

    def fin_job():
        acc_buf[...] = lane_sum(acc_buf[...])
        l_buf[...] = g_buf[0] / lane_sum(l_buf[...])
        m_buf[_HQ - 1] = lane_max(m_buf[_HQ - 1])

    def tiles_dot(buf, col, row, nt):
        w = buf[pl.ds(row, nt * BR), :].astype(f32).reshape(nt, DB, 8, _LN)
        return jnp.sum(w * col[:, None], axis=0)

    OJ = 4
    OT = RT // OJ

    def o_job(h, k):
        col = acc_buf[pl.ds(k * OT, OT)]
        a_buf[...] += (tiles_dot(wo_buf, col, mo((h * OJ + k) * (OT * BR), 16), OT)
                       * l_buf[...][None])

    def f_job(j):
        ch = srl(j, 1)
        up = jnp.bitwise_and(j, 1)
        x8 = jnp.concatenate([x8_buf[t] for t in range(DB)], axis=1).astype(bf16)
        t = jnp.dot(x8, wgu_buf[up, :, pl.ds(mo(ch * _LN, _LN), _LN)], preferred_element_type=f32)
        h_buf[ch] = jnp.where(up == 1, jax.nn.silu(h_buf[ch]), 1.0) * t

    def c_job(ch):
        hc_buf[pl.ds(ch * BT, BT)] = columns(h_buf[ch] * g_buf[1])

    def d_job(ch):
        a_buf[...] += tiles_dot(wd_buf, hc_buf[pl.ds(ch * BT, BT)], mo(ch * (BT * BR), 16), BT)

    DP = FB + 1
    assert DP + WD_B < _HQ and OC + 1 + OJ + 3 <= NC and OC + 1 + OJ <= D1

    def v_period(h, st):
        with scope("vper"):
            e, l, acc = st
            first = (h >= 1).astype(jnp.int32)
            nf = jnp.where(h < FB, 2, 0)
            nc = jnp.logical_and(h >= 1, h < DP).astype(jnp.int32)
            nd = jnp.logical_and(h >= DP, h < DP + WD_B).astype(jnp.int32)
            acc_buf[...] = acc
            l_buf[...] = l
            st = (e, jnp.zeros((8, _LN), f32), jnp.zeros((RT, 8, _LN), f32))
            st = jax.lax.fori_loop(0, OC, lambda c, st: v_slot(h, c, st), st)
            st = v_slot(h, jnp.int32(OC), st, fin_job)

            @pl.when(h >= 1)
            def _():
                wait_all(wo_buf.at[pl.ds(mo((h - 1) * (RT * BR), 64), RT * BR)], sem_wo.at[h - 1])
            c1 = OC + 1 + first * OJ
            st = jax.lax.fori_loop(
                OC + 1, c1, lambda c, st: v_slot(h, c, st, lambda: o_job(h - 1, c - OC - 1)), st)

            @pl.when(h == 0)
            def _():
                wait_all(wgu_buf, sem_gu.at[0])
            c2 = c1 + nf
            st = jax.lax.fori_loop(
                c1, c2, lambda c, st: v_slot(h, c, st, lambda: f_job(2 * h + c - c1)), st)
            c3 = c2 + nc
            st = jax.lax.fori_loop(c2, c3, lambda c, st: v_slot(h, c, st, lambda: c_job(h - 1)), st)

            @pl.when(h == DP)
            def _():
                wait_all(wd_buf.at[band_rows(0, TB)], sem_wd.at[0])
            c4 = c3 + nd
            st = jax.lax.fori_loop(c3, c4, lambda c, st: v_slot(h, c, st, lambda: d_job(h - DP)), st)
            st = jax.lax.fori_loop(c4, jnp.where(h == _HQ - 1, NC - D1, NC),
                                   lambda c, st: v_slot(h, c, st), st)
        return st
    st = (e0, jnp.ones((8, _LN), f32), jnp.zeros((RT, 8, _LN), f32))
    st = jax.lax.fori_loop(0, _HQ, v_period, st)

    def group_copy(i):
        sl = band_rows(*groups[i])
        return pltpu.make_async_copy(wd_hbm.at[sl], wd_buf.at[sl], sem_wd.at[1 + i])

    with scope("vlast"):
        for i in range(2, len(groups)):
            group_copy(i).start(priority=1)
        e, l, acc = jax.lax.fori_loop(
            NC - D1, NC - 1, lambda c, st: v_slot(_HQ - 1, c, st, tail=True), st)

    with scope("tail"):
        wait_all(wo_buf.at[pl.ds((_HQ - 1) * RT * BR, RT * BR)], sem_wo.at[_HQ - 1])
        gate = g_buf[0]
        inv = gate / lane_sum(l + e)
        base = []
        for cb in range(DB):
            xt = x8_buf[cb]
            base.append(((1.0 - gate) * (xt + xt * 0.0))[0:1])
        wait_all(ring.at[NC - 1], sem_ring.at[NC - 1])
        if TQ0 == D1:
            tq0_start(D1 - 1)
        col = lane_sum(pv_add(acc, e, NC - 1))
        a = a_buf[...] + tiles_dot(wo_buf, col, (_HQ - 1) * RT * BR, RT) * inv[None]
        for i in ORDER:
            b0, nb = groups[i]
            group_copy(i).wait()
            a = a + tiles_dot(wd_buf, hc_buf[pl.ds(b0, nb)], b0 * BR, nb)
        res = [base[cb] + jnp.sum(a[cb], axis=0, keepdims=True) for cb in range(DB)]
        o_ref[...] = jnp.concatenate(res, axis=1).astype(o_ref.dtype)


def _build(D1=16, SCOPES=False, TQ0=10, TQA=10, TAILP=(22, 10, 4, 2), ORDER=(0, 2, 3, 4, 5),
           OC=8, ST=256, SPLIT=True, JC=8):
    def fn(A_x, A_k_cache, A_v_cache, A_wq, A_wo, B_x, B_w_r, B_w_gate, B_w_up, B_w_down, gate_w):
        B, Sq, D = A_x.shape
        _, Hkv, SK, Dh = A_k_cache.shape
        assert B == 1 and Sq == 1 and Hkv == _HQ and Dh == _DH
        W = min(4096, max(256, SK // 4))
        F = B_w_gate.shape[1]
        n_rows = _HQ * _DH
        NC = W // _LN
        DB, FB = D // _LN, F // _LN
        bf16, f32 = jnp.bfloat16, jnp.float32

        def tiles(w, st=1):
            r, c = w.shape
            t = w.reshape(r // 8, 8, c // _LN, _LN).transpose(0, 2, 1, 3)
            n = (r // 8) * (c // _LN) // st
            return t.reshape(n, st, 8, _LN).transpose(0, 2, 1, 3).reshape(n * 8, st * _LN)

        x = A_x.reshape(1, D)
        kt = jnp.swapaxes(A_k_cache, 2, 3).reshape(n_rows, SK)
        vt = jnp.swapaxes(A_v_cache, 2, 3).reshape(n_rows, SK)
        wr = B_w_r.reshape(DB, _LN)
        gw = gate_w.reshape(DB, _LN)
        wq = tiles(A_wq, ST)

        any_spec = pl.BlockSpec(memory_space=pl.ANY)
        out = pl.pallas_call(
            functools.partial(_kernel, D1=D1, W=W, SK=SK, D=D, F=F, ST=ST, SCOPES=SCOPES, TQ0=TQ0,
                              TQA=TQA, TAILP=TAILP, ORDER=ORDER, SPLIT=SPLIT, OC=OC, JC=JC),
            in_specs=[any_spec] * 10,
            out_specs=pl.BlockSpec(memory_space=pltpu.VMEM),
            out_shape=jax.ShapeDtypeStruct((1, D), bf16),
            scratch_shapes=[
                pltpu.VMEM((1, D), bf16),
                pltpu.VMEM((2, DB, _LN), bf16),
                pltpu.VMEM((ST // 2, wq.shape[0], 2 * _LN), bf16),
                pltpu.VMEM((2, D, F), bf16),
                pltpu.VMEM((n_rows * DB, _LN), bf16),
                pltpu.VMEM((F * DB, _LN), bf16),
                pltpu.VMEM((NC, _DH, _LN), bf16),
                pltpu.VMEM((DB, 8, _LN), f32),
                pltpu.VMEM((D // 8, 8, _LN), f32),
                pltpu.VMEM((2, 8, _LN), f32),
                pltpu.VMEM((n_rows // _LN, 8, _LN), f32),
                pltpu.VMEM((n_rows // 8, 8, _LN), f32),
                pltpu.VMEM((_HQ * NC, 8, _LN), f32),
                pltpu.VMEM((_HQ, 8, _LN), f32),
                pltpu.VMEM((_DH // 8, 8, _LN), f32),
                pltpu.VMEM((8, _LN), f32),
                pltpu.VMEM((FB, 8, _LN), f32),
                pltpu.VMEM((F // 8, 8, _LN), f32),
                pltpu.VMEM((DB, 8, _LN), f32),
                pltpu.SemaphoreType.DMA((3,)),
                pltpu.SemaphoreType.DMA((1,)),
                pltpu.SemaphoreType.DMA((_HQ,)),
                pltpu.SemaphoreType.DMA((3 + len(TAILP),)),
                pltpu.SemaphoreType.DMA((NC,)),
            ],
            compiler_params=_compiler_params(vmem_limit_bytes=100 * 1024 * 1024,
                                             disable_bounds_checks=True,
                                             disable_semaphore_checks=True),
        )(x, kt, vt, wq, tiles(A_wo), wr, B_w_gate, B_w_up, tiles(B_w_down), gw)
        return out.reshape(B, Sq, D)
    return fn


@jax.jit
def pallas_gated_mix__sliding_block_cached__moe_arch_mod__decode_kernel(
    A_x: jax.Array,
    A_k_cache: jax.Array,
    A_v_cache: jax.Array,
    A_wq: jax.Array,
    A_wo: jax.Array,
    B_x: jax.Array,
    B_w_r: jax.Array,
    B_w_gate: jax.Array,
    B_w_up: jax.Array,
    B_w_down: jax.Array,
    gate_w: jax.Array,
):
    return _build()(A_x, A_k_cache, A_v_cache, A_wq, A_wo, B_x, B_w_r,
                    B_w_gate, B_w_up, B_w_down, gate_w)
```

```python
import dataclasses
import functools
import math

import jax
import jax.numpy as jnp
import jax.experimental.pallas as pl
import jax.experimental.pallas.tpu as pltpu

_HQ = 32
_DH = 192
_LN = 128


def _const_div(n, d, hi):
    if isinstance(n, int):
        return n // d
    for sh in range(1, 20):
        m = -(-(1 << sh) // d)
        if all((v * m) >> sh == v // d for v in range(hi)):
            return jax.lax.shift_right_logical(n * m, sh)
    raise ValueError("no multiplier")


def _compiler_params(**kw):
    names = {f.name for f in dataclasses.fields(pltpu.CompilerParams)}
    return pltpu.CompilerParams(**{k: v for k, v in kw.items() if k in names})


class _NoScope:
    def __enter__(self):
        return self

    def __exit__(self, *a):
        return False


def _kernel(x_hbm, k_hbm, v_hbm, wq_hbm, wo_hbm, wr_hbm, wg_hbm, wu_hbm, wd_hbm, gw_hbm,
            o_ref,
            x_buf, small_buf, wq_buf, wgu_buf, wo_buf, wd_buf, ring,
            x8_buf, xc_buf, g_buf, q_buf, qc_buf, s_buf, m_buf, acc_buf, l_buf, h_buf, hc_buf,
            a_buf,
            sem_small, sem_wq, sem_gu, sem_wo, sem_wd, sem_ring,
            *, D1, W, SK, D, F, ST, SCOPES, TQ0, TQA, TAILP, ORDER, OC, JC):
    f32, bf16 = jnp.float32, jnp.bfloat16
    scope = jax.named_scope if SCOPES else (lambda name: _NoScope())
    NC = W // _LN
    NS = _HQ * NC
    DB = D // _LN
    FB = F // _LN
    QB = _HQ * _DH // _LN
    RT = _DH // 8
    BT = _LN // 8
    col0 = SK - W
    assert NC == 32 and D1 == NC // 2 and D % _LN == 0 and F % _LN == 0
    WB = (D // 8) * QB // ST
    WC = 2 * _LN
    NW = ST // 2
    WR = QB // math.gcd(ST, QB)
    WK = WR * ST // QB
    assert WB * ST == (D // 8) * QB and WB % WR == 0 and NW % NC == 0 and QB % 2 == 0
    PT = 3
    GP = FB // PT
    N_WG = (D // 8) * GP
    WD_B = 9
    DT = 2
    N_WD = WD_B * BT * DB // DT
    WD_W = 2 * NW - (DB + 1)
    S_WG = NW + 2 + N_WD - WD_W
    S_WU = S_WG + N_WG
    S_WO = S_WU + N_WG
    OP = RT * DB // PT
    S_V = NW + NS
    assert GP == 4 and FB % PT == 0 and (WD_B * BT * DB) % DT == 0 and (RT * DB) % PT == 0
    assert S_WO + _HQ * OP == S_V + NS - D1 and S_WO < S_V - D1
    scale = _DH ** -0.5

    def mo(v, m):
        return v if isinstance(v, int) else pl.multiple_of(v, m)
    srl = jax.lax.shift_right_logical

    def kv_start(src, t):
        row = mo((t >> 5) * _DH, _DH // 3)
        c = t & (NC - 1)
        col = mo(col0 + c * _LN, _LN)
        pltpu.make_async_copy(src.at[pl.ds(row, _DH), pl.ds(col, _LN)],
                              ring.at[c], sem_ring.at[c]).start(priority=1)

    def wq_dst(j, i):
        return wq_buf.at[j, :, pl.ds(i * _LN, _LN)], sem_wq.at[(2 * j + i) & (2 * D1 - 1)]

    def wq_start(j, i):
        pltpu.make_async_copy(wq_hbm.at[:, pl.ds(mo(j * WC + i * _LN, _LN), _LN)],
                              *wq_dst(j, i)).start(priority=1)

    def wait_all(ref, sem):
        pltpu.make_async_copy(ref, ref, sem).wait()

    def gu_start(src, i, u):
        sl = (pl.ds(mo((u >> 2) * 8, 8), 8), pl.ds(mo((u & 3) * (PT * _LN), _LN), PT * _LN))
        pltpu.make_async_copy(src.at[sl], wgu_buf.at[i].at[sl], sem_gu.at[0]).start(priority=0)

    def wg_start(g):
        gu_start(wg_hbm, 0, g - S_WG)

    def wu_start(g):
        gu_start(wu_hbm, 1, g - S_WU)

    def wd_piece(u):
        sl = pl.ds(mo(u * (DT * 8), DT * 8), DT * 8)
        pltpu.make_async_copy(wd_hbm.at[sl], wd_buf.at[sl], sem_wd.at[0]).start(priority=0)

    def wd_start(g):
        wd_piece(g - S_WG + N_WD)

    def wo_start(g):
        u = g - S_WO
        sl = pl.ds(mo(u * (PT * 8), 8), PT * 8)
        pltpu.make_async_copy(wo_hbm.at[sl], wo_buf.at[sl],
                              sem_wo.at[_const_div(u, OP, _HQ * OP)]).start(priority=0)

    BR = DB * 8
    TB = WD_B * BT

    def band_rows(b0, nb):
        return pl.ds(mo(b0 * BR, 8), nb * BR)

    def tq0_start(i):
        sl = band_rows(TB + i, 1)
        k = int(i >= TQA) if isinstance(i, int) else (i >= TQA).astype(jnp.int32)
        pltpu.make_async_copy(wd_hbm.at[sl], wd_buf.at[sl], sem_wd.at[1 + k]).start(priority=0)

    groups = [(TB, TQA), (TB + TQA, TQ0 - TQA)]
    for nb in TAILP:
        groups.append((sum(groups[-1]), nb))
    assert sum(groups[-1]) == F // 8 and all(b % 2 == 0 and n % 2 == 0 for b, n in groups)
    assert sorted(ORDER) == [i for i, (_, n) in enumerate(groups) if n] and TQ0 <= D1

    x_cp = pltpu.make_async_copy(x_hbm, x_buf, sem_small.at[0])
    wr_cp = pltpu.make_async_copy(wr_hbm, small_buf.at[0], sem_small.at[1])
    gw_cp = pltpu.make_async_copy(gw_hbm, small_buf.at[1], sem_small.at[2])
    wq_start(0, 0)
    x_cp.start(priority=0)
    for j in range(1, 2 * D1):
        wq_start(j >> 1, j & 1)
    wr_cp.start(priority=0)
    gw_cp.start(priority=0)
    a_buf[...] = jnp.zeros(a_buf.shape, f32)
    q_buf[...] = jnp.zeros(q_buf.shape, f32)
    h_buf[...] = jnp.zeros(h_buf.shape, f32)

    lane_id = jax.lax.broadcasted_iota(jnp.int32, (8, _LN), 1)
    diag = lane_id - jax.lax.broadcasted_iota(jnp.int32, (8, _LN), 0)

    def lane_sum(v):
        return jnp.broadcast_to(jnp.sum(v, axis=-1, keepdims=True), v.shape)

    def columns(v):
        return lane_sum(jnp.stack([jnp.where(diag == 8 * k, v, 0.0) for k in range(BT)]))

    def loop(lo, hi, body):
        def b(n, c):
            body(n)
            return c
        jax.lax.fori_loop(lo, hi, b, 0)

    def q_add(j):
        w = wq_buf[j].astype(f32)
        for r in range(WR):
            p = r * NW + j
            kb = _const_div(p, QB // 2, WR * NW)
            cb = 2 * p - QB * kb
            xc = [xc_buf[kb + WK * i] for i in range(WB // WR)]
            for jj in range(2):
                acc = q_buf[cb + jj]
                for i in range(WB // WR):
                    b = r + WR * i
                    acc = acc + w[8 * b:8 * b + 8, jj * _LN:(jj + 1) * _LN] * xc[i]
                q_buf[cb + jj] = acc

    def w_slot(j, u, job, nxt=False, both=True):
        for i in range(2):
            wait_all(*wq_dst(j, i))
            if both or i == 0:
                wd_piece(u + i)
            if not nxt:
                wq_start(j + D1, i)
            elif i == 1:
                kv_start(k_hbm, j + D1 - NW)
        job()

    def x_job(t):
        if t == 0:
            x_cp.wait()
        xt = jnp.broadcast_to(x_buf[:, t * _LN:(t + 1) * _LN].astype(f32), (8, _LN))
        x8_buf[t] = xt
        xc_buf[pl.ds(t * BT, BT)] = columns(xt)

    def gate_job():
        wr_cp.wait()
        gw_cp.wait()
        wr = small_buf[0].astype(f32)
        gw = small_buf[1].astype(f32)
        r_acc = jnp.zeros((8, _LN), f32)
        g_acc = jnp.zeros((8, _LN), f32)
        for t in range(DB):
            xt = x8_buf[t]
            r_acc = r_acc + xt * jnp.broadcast_to(wr[t:t + 1, :], (8, _LN))
            g_acc = g_acc + xt * jnp.broadcast_to(gw[t:t + 1, :], (8, _LN))
        r_sel = jax.nn.sigmoid(lane_sum(r_acc))
        gate = jax.nn.sigmoid(lane_sum(g_acc))
        g_buf[0] = gate
        g_buf[1] = (1.0 - gate) * r_sel

    with scope("w0"):
        for t in range(DB):
            w_slot(t, t, functools.partial(x_job, t), both=False)

        def two(j):
            q_add(j - DB)
            q_add(j)
        loop(DB, 2 * DB, lambda j: w_slot(j, 2 * j - DB, lambda: two(j)))

        def with_gate():
            gate_job()
            q_add(2 * DB)
        w_slot(2 * DB, 3 * DB, with_gate, both=False)
    with scope("w1"):
        loop(2 * DB + 1, NW - D1, lambda j: w_slot(j, 2 * j - DB - 1, lambda: q_add(j)))
        loop(NW - D1, NW, lambda j: w_slot(j, 2 * j - DB - 1, lambda: q_add(j), nxt=True))

    def row_sum(v):
        return jnp.broadcast_to(jnp.sum(v, axis=0, keepdims=True), (8, _LN))

    def q_fin(h):
        odd = h & 1
        cb = (3 * h) >> 1
        va, vb = row_sum(q_buf[cb]), row_sum(q_buf[cb + 1])
        vm = jnp.where(odd == 1, vb, va)
        lo, hi = diag - 64 * odd, diag + 64 * odd
        t = ([jnp.where(lo == 8 * r, va, 0.0) for r in range(8)]
             + [jnp.where(hi == 8 * r, vm, 0.0) for r in range(8, 16)]
             + [jnp.where(lo == 8 * r, vb, 0.0) for r in range(8)])
        qc_buf[pl.ds(h * RT, RT)] = lane_sum(jnp.stack(t))

    def lane_max(m):
        return jnp.broadcast_to(jnp.max(m, axis=-1, keepdims=True), (8, _LN))

    def score(t):
        p = (ring[t & (NC - 1)].astype(f32).reshape(RT // 4, 4, 8, _LN)
             * qc_buf[pl.ds((t >> 5) * RT, RT)].reshape(RT // 4, 4, 8, _LN))
        p = jnp.sum(p, axis=0)
        s = row_sum((p[0] + p[1]) + (p[2] + p[3]))
        s_buf[t] = s
        return s

    def k_dma(q0, nxt, t):
        c = t & (NC - 1)
        wait_all(ring.at[c], sem_ring.at[c])
        if q0 is not None:
            q0(NW + t)
        if nxt:
            kv_start(v_hbm, t + D1 - NS)
        else:
            kv_start(k_hbm, t + D1)

    def k_slot(q0, nxt, t, m):
        c = t & (NC - 1)
        h = srl(t, 5)
        k_dma(q0, nxt, t)
        m = jnp.maximum(jnp.where(c == 0, -jnp.inf, m), score(t))
        m_buf[h] = m

        @pl.when(c == JC)
        def _():
            hp = jnp.maximum(h - 1, 0)
            m_buf[hp] = lane_max(m_buf[hp])
            q_fin(jnp.minimum(h + 1, _HQ - 1))
        return m

    k_dma(None, False, 0)
    q_fin(0)
    k_dma(None, False, 1)
    m = jnp.maximum(score(0), score(1))
    lo = NW + 2
    for hi, q0, nxt in ((S_WG, wd_start, False), (S_WU, wg_start, False), (S_WO, wu_start, False),
                        (S_V - D1, wo_start, False), (S_V, wo_start, True)):
        if nxt:
            e0 = jnp.exp((s_buf[0] - m_buf[0]) * scale)
        with scope("k%d" % lo):
            m = jax.lax.fori_loop(lo - NW, hi - NW, functools.partial(k_slot, q0, nxt), m)
        lo = hi

    def prob(n):
        return jnp.exp((s_buf[n] - m_buf[srl(n, 5)]) * scale)

    def pv_add(acc, e, c):
        return acc + ring[c].astype(f32).reshape(RT, 8, _LN) * e[None]

    def v_slot(h, c, st, job=None, tail=False):
        e, l, acc = st
        n = h * NC + c
        wait_all(ring.at[c], sem_ring.at[c])
        if tail:
            if TQ0 >= D1 - 1:
                tq0_start(c - D1)
            else:
                @pl.when(c - D1 < TQ0)
                def _():
                    tq0_start(c - D1)
        else:
            wo_start(S_V + n)
            kv_start(v_hbm, n + D1)
        acc = pv_add(acc, e, c)
        if job is not None:
            job()
        return prob(n + 1), l + e, acc

    def fin_job():
        acc_buf[...] = lane_sum(acc_buf[...])
        l_buf[...] = g_buf[0] / lane_sum(l_buf[...])
        m_buf[_HQ - 1] = lane_max(m_buf[_HQ - 1])

    def tiles_dot(buf, col, row, nt):
        w = buf[pl.ds(row, nt * BR), :].astype(f32).reshape(nt, DB, 8, _LN)
        return jnp.sum(w * col[:, None], axis=0)

    OJ = 4
    OT = RT // OJ

    def o_job(h, k):
        col = acc_buf[pl.ds(k * OT, OT)]
        a_buf[...] += (tiles_dot(wo_buf, col, mo((h * OJ + k) * (OT * BR), 16), OT)
                       * l_buf[...][None])

    def f_job(j):
        ch = srl(j, 1)
        up = jnp.bitwise_and(j, 1)
        x8 = jnp.concatenate([x8_buf[t] for t in range(DB)], axis=1).astype(bf16)
        t = jnp.dot(x8, wgu_buf[up, :, pl.ds(mo(ch * _LN, _LN), _LN)], preferred_element_type=f32)
        h_buf[ch] = jnp.where(up == 1, jax.nn.silu(h_buf[ch]), 1.0) * t

    def c_job(ch):
        hc_buf[pl.ds(ch * BT, BT)] = columns(h_buf[ch] * g_buf[1])

    def d_job(ch):
        a_buf[...] += tiles_dot(wd_buf, hc_buf[pl.ds(ch * BT, BT)], mo(ch * (BT * BR), 16), BT)

    DP = FB + 1
    assert DP + WD_B < _HQ and OC + 1 + OJ + 3 <= NC and OC + 1 + OJ <= D1

    def v_period(h, st):
        with scope("vper"):
            e, l, acc = st
            first = (h >= 1).astype(jnp.int32)
            nf = jnp.where(h < FB, 2, 0)
            nc = jnp.logical_and(h >= 1, h < DP).astype(jnp.int32)
            nd = jnp.logical_and(h >= DP, h < DP + WD_B).astype(jnp.int32)
            acc_buf[...] = acc
            l_buf[...] = l
            st = (e, jnp.zeros((8, _LN), f32), jnp.zeros((RT, 8, _LN), f32))
            st = jax.lax.fori_loop(0, OC, lambda c, st: v_slot(h, c, st), st)
            st = v_slot(h, jnp.int32(OC), st, fin_job)

            @pl.when(h >= 1)
            def _():
                wait_all(wo_buf.at[pl.ds(mo((h - 1) * (RT * BR), 64), RT * BR)], sem_wo.at[h - 1])
            c1 = OC + 1 + first * OJ
            st = jax.lax.fori_loop(
                OC + 1, c1, lambda c, st: v_slot(h, c, st, lambda: o_job(h - 1, c - OC - 1)), st)

            @pl.when(h == 0)
            def _():
                wait_all(wgu_buf, sem_gu.at[0])
            c2 = c1 + nf
            st = jax.lax.fori_loop(
                c1, c2, lambda c, st: v_slot(h, c, st, lambda: f_job(2 * h + c - c1)), st)
            c3 = c2 + nc
            st = jax.lax.fori_loop(c2, c3, lambda c, st: v_slot(h, c, st, lambda: c_job(h - 1)), st)

            @pl.when(h == DP)
            def _():
                wait_all(wd_buf.at[band_rows(0, TB)], sem_wd.at[0])
            c4 = c3 + nd
            st = jax.lax.fori_loop(c3, c4, lambda c, st: v_slot(h, c, st, lambda: d_job(h - DP)), st)
            st = jax.lax.fori_loop(c4, jnp.where(h == _HQ - 1, NC - D1, NC),
                                   lambda c, st: v_slot(h, c, st), st)
        return st
    st = (e0, jnp.ones((8, _LN), f32), jnp.zeros((RT, 8, _LN), f32))
    st = jax.lax.fori_loop(0, _HQ, v_period, st)

    def group_copy(i):
        sl = band_rows(*groups[i])
        return pltpu.make_async_copy(wd_hbm.at[sl], wd_buf.at[sl], sem_wd.at[1 + i])

    with scope("vlast"):
        for i in range(2, len(groups)):
            group_copy(i).start(priority=1)
        e, l, acc = jax.lax.fori_loop(
            NC - D1, NC - 1, lambda c, st: v_slot(_HQ - 1, c, st, tail=True), st)

    with scope("tail"):
        wait_all(wo_buf.at[pl.ds((_HQ - 1) * RT * BR, RT * BR)], sem_wo.at[_HQ - 1])
        gate = g_buf[0]
        inv = gate / lane_sum(l + e)
        base = []
        for cb in range(DB):
            xt = x8_buf[cb]
            base.append(((1.0 - gate) * (xt + xt * 0.0))[0:1])
        wait_all(ring.at[NC - 1], sem_ring.at[NC - 1])
        if TQ0 == D1:
            tq0_start(D1 - 1)
        col = lane_sum(pv_add(acc, e, NC - 1))
        a = a_buf[...] + tiles_dot(wo_buf, col, (_HQ - 1) * RT * BR, RT) * inv[None]
        for i in ORDER:
            b0, nb = groups[i]
            group_copy(i).wait()
            a = a + tiles_dot(wd_buf, hc_buf[pl.ds(b0, nb)], b0 * BR, nb)
        res = [base[cb] + jnp.sum(a[cb], axis=0, keepdims=True) for cb in range(DB)]
        o_ref[...] = jnp.concatenate(res, axis=1).astype(o_ref.dtype)


def _build(D1=16, SCOPES=False, TQ0=10, TQA=10, TAILP=(22, 10, 4, 2), ORDER=(0, 2, 3, 4, 5),
           OC=8, ST=256, JC=8):
    def fn(A_x, A_k_cache, A_v_cache, A_wq, A_wo, B_x, B_w_r, B_w_gate, B_w_up, B_w_down, gate_w):
        B, Sq, D = A_x.shape
        _, Hkv, SK, Dh = A_k_cache.shape
        assert B == 1 and Sq == 1 and Hkv == _HQ and Dh == _DH
        W = min(4096, max(256, SK // 4))
        F = B_w_gate.shape[1]
        n_rows = _HQ * _DH
        NC = W // _LN
        DB, FB = D // _LN, F // _LN
        bf16, f32 = jnp.bfloat16, jnp.float32

        def tiles(w, st=1):
            r, c = w.shape
            t = w.reshape(r // 8, 8, c // _LN, _LN).transpose(0, 2, 1, 3)
            n = (r // 8) * (c // _LN) // st
            return t.reshape(n, st, 8, _LN).transpose(0, 2, 1, 3).reshape(n * 8, st * _LN)

        x = A_x.reshape(1, D)
        kt = jnp.swapaxes(A_k_cache, 2, 3).reshape(n_rows, SK)
        vt = jnp.swapaxes(A_v_cache, 2, 3).reshape(n_rows, SK)
        wr = B_w_r.reshape(DB, _LN)
        gw = gate_w.reshape(DB, _LN)
        wq = tiles(A_wq, ST)

        any_spec = pl.BlockSpec(memory_space=pl.ANY)
        out = pl.pallas_call(
            functools.partial(_kernel, D1=D1, W=W, SK=SK, D=D, F=F, ST=ST, SCOPES=SCOPES, TQ0=TQ0,
                              TQA=TQA, TAILP=TAILP, ORDER=ORDER, OC=OC, JC=JC),
            in_specs=[any_spec] * 10,
            out_specs=pl.BlockSpec(memory_space=pltpu.VMEM),
            out_shape=jax.ShapeDtypeStruct((1, D), bf16),
            scratch_shapes=[
                pltpu.VMEM((1, D), bf16),
                pltpu.VMEM((2, DB, _LN), bf16),
                pltpu.VMEM((ST // 2, wq.shape[0], 2 * _LN), bf16),
                pltpu.VMEM((2, D, F), bf16),
                pltpu.VMEM((n_rows * DB, _LN), bf16),
                pltpu.VMEM((F * DB, _LN), bf16),
                pltpu.VMEM((NC, _DH, _LN), bf16),
                pltpu.VMEM((DB, 8, _LN), f32),
                pltpu.VMEM((D // 8, 8, _LN), f32),
                pltpu.VMEM((2, 8, _LN), f32),
                pltpu.VMEM((n_rows // _LN, 8, _LN), f32),
                pltpu.VMEM((n_rows // 8, 8, _LN), f32),
                pltpu.VMEM((_HQ * NC, 8, _LN), f32),
                pltpu.VMEM((_HQ, 8, _LN), f32),
                pltpu.VMEM((_DH // 8, 8, _LN), f32),
                pltpu.VMEM((8, _LN), f32),
                pltpu.VMEM((FB, 8, _LN), f32),
                pltpu.VMEM((F // 8, 8, _LN), f32),
                pltpu.VMEM((DB, 8, _LN), f32),
                pltpu.SemaphoreType.DMA((3,)),
                pltpu.SemaphoreType.DMA((2 * D1,)),
                pltpu.SemaphoreType.DMA((1,)),
                pltpu.SemaphoreType.DMA((_HQ,)),
                pltpu.SemaphoreType.DMA((3 + len(TAILP),)),
                pltpu.SemaphoreType.DMA((NC,)),
            ],
            compiler_params=_compiler_params(vmem_limit_bytes=100 * 1024 * 1024,
                                             disable_bounds_checks=True,
                                             disable_semaphore_checks=True),
        )(x, kt, vt, wq, tiles(A_wo), wr, B_w_gate, B_w_up, tiles(B_w_down), gw)
        return out.reshape(B, Sq, D)
    return fn


@jax.jit
def pallas_gated_mix__sliding_block_cached__moe_arch_mod__decode_kernel(
    A_x: jax.Array,
    A_k_cache: jax.Array,
    A_v_cache: jax.Array,
    A_wq: jax.Array,
    A_wo: jax.Array,
    B_x: jax.Array,
    B_w_r: jax.Array,
    B_w_gate: jax.Array,
    B_w_up: jax.Array,
    B_w_down: jax.Array,
    gate_w: jax.Array,
):
    return _build()(A_x, A_k_cache, A_v_cache, A_wq, A_wo, B_x, B_w_r,
                    B_w_gate, B_w_up, B_w_down, gate_w)
```

```python
import dataclasses
import functools
import math

import jax
import jax.numpy as jnp
import jax.experimental.pallas as pl
import jax.experimental.pallas.tpu as pltpu

_HQ = 32
_DH = 192
_LN = 128


def _const_div(n, d, hi):
    if isinstance(n, int):
        return n // d
    for sh in range(1, 20):
        m = -(-(1 << sh) // d)
        if all((v * m) >> sh == v // d for v in range(hi)):
            return jax.lax.shift_right_logical(n * m, sh)
    raise ValueError("no multiplier")


def _compiler_params(**kw):
    names = {f.name for f in dataclasses.fields(pltpu.CompilerParams)}
    return pltpu.CompilerParams(**{k: v for k, v in kw.items() if k in names})


class _NoScope:
    def __enter__(self):
        return self

    def __exit__(self, *a):
        return False


def _kernel(x_hbm, k_hbm, v_hbm, wq_hbm, wo_hbm, wr_hbm, wg_hbm, wu_hbm, wd_hbm, gw_hbm,
            o_ref,
            x_buf, small_buf, wq_buf, wgu_buf, wo_buf, wd_buf, ring,
            x8_buf, xc_buf, g_buf, q_buf, qc_buf, s_buf, m_buf, acc_buf, l_buf, h_buf, hc_buf,
            a_buf,
            sem_small, sem_wq, sem_gu, sem_wo, sem_wd, sem_ring,
            *, D1, W, SK, D, F, ST, SCOPES, TQ0, TQA, TAILP, ORDER, OC, JC):
    f32, bf16 = jnp.float32, jnp.bfloat16
    scope = jax.named_scope if SCOPES else (lambda name: _NoScope())
    NC = W // _LN
    NS = _HQ * NC
    DB = D // _LN
    FB = F // _LN
    QB = _HQ * _DH // _LN
    RT = _DH // 8
    BT = _LN // 8
    col0 = SK - W
    assert NC == 32 and D1 == NC // 2 and D % _LN == 0 and F % _LN == 0
    WB = (D // 8) * QB // ST
    WC = 2 * _LN
    NW = ST // 2
    WR = QB // math.gcd(ST, QB)
    WK = WR * ST // QB
    assert WB * ST == (D // 8) * QB and WB % WR == 0 and NW % NC == 0 and QB % 2 == 0
    PT = 3
    GP = FB // PT
    N_WG = (D // 8) * GP
    WD_B = 9
    DT = 2
    N_WD = WD_B * BT * DB // DT
    WD_W = 2 * NW - (DB + 3)
    S_WG = NW + N_WD - WD_W
    S_WU = S_WG + N_WG
    S_WO = S_WU + N_WG
    OP = RT * DB // PT
    S_V = NW + NS
    assert GP == 4 and FB % PT == 0 and (WD_B * BT * DB) % DT == 0 and (RT * DB) % PT == 0
    assert S_WO + _HQ * OP == S_V + NS - D1 and S_WO < S_V - D1
    scale = _DH ** -0.5

    def mo(v, m):
        return v if isinstance(v, int) else pl.multiple_of(v, m)
    srl = jax.lax.shift_right_logical

    def kv_start(src, t):
        row = mo((t >> 5) * _DH, _DH // 3)
        c = t & (NC - 1)
        col = mo(col0 + c * _LN, _LN)
        pltpu.make_async_copy(src.at[pl.ds(row, _DH), pl.ds(col, _LN)],
                              ring.at[c], sem_ring.at[c]).start(priority=1)

    def wq_dst(j, i):
        return wq_buf.at[j, :, pl.ds(i * _LN, _LN)], sem_wq.at[(2 * j + i) & (2 * D1 - 1)]

    def wq_start(j, i):
        pltpu.make_async_copy(wq_hbm.at[:, pl.ds(mo(j * WC + i * _LN, _LN), _LN)],
                              *wq_dst(j, i)).start(priority=1)

    def wait_all(ref, sem):
        pltpu.make_async_copy(ref, ref, sem).wait()

    def gu_start(src, i, u):
        sl = (pl.ds(mo((u >> 2) * 8, 8), 8), pl.ds(mo((u & 3) * (PT * _LN), _LN), PT * _LN))
        pltpu.make_async_copy(src.at[sl], wgu_buf.at[i].at[sl], sem_gu.at[0]).start(priority=0)

    def wg_start(g):
        gu_start(wg_hbm, 0, g - S_WG)

    def wu_start(g):
        gu_start(wu_hbm, 1, g - S_WU)

    def wd_piece(u):
        sl = pl.ds(mo(u * (DT * 8), DT * 8), DT * 8)
        pltpu.make_async_copy(wd_hbm.at[sl], wd_buf.at[sl], sem_wd.at[0]).start(priority=0)

    def wd_start(g):
        wd_piece(g - S_WG + N_WD)

    def wo_start(g):
        u = g - S_WO
        sl = pl.ds(mo(u * (PT * 8), 8), PT * 8)
        pltpu.make_async_copy(wo_hbm.at[sl], wo_buf.at[sl],
                              sem_wo.at[_const_div(u, OP, _HQ * OP)]).start(priority=0)

    BR = DB * 8
    TB = WD_B * BT

    def band_rows(b0, nb):
        return pl.ds(mo(b0 * BR, 8), nb * BR)

    def tq0_start(i):
        sl = band_rows(TB + i, 1)
        k = int(i >= TQA) if isinstance(i, int) else (i >= TQA).astype(jnp.int32)
        pltpu.make_async_copy(wd_hbm.at[sl], wd_buf.at[sl], sem_wd.at[1 + k]).start(priority=0)

    groups = [(TB, TQA), (TB + TQA, TQ0 - TQA)]
    for nb in TAILP:
        groups.append((sum(groups[-1]), nb))
    assert sum(groups[-1]) == F // 8 and all(b % 2 == 0 and n % 2 == 0 for b, n in groups)
    assert sorted(ORDER) == [i for i, (_, n) in enumerate(groups) if n] and TQ0 <= D1

    x_cp = pltpu.make_async_copy(x_hbm, x_buf, sem_small.at[0])
    wr_cp = pltpu.make_async_copy(wr_hbm, small_buf.at[0], sem_small.at[1])
    gw_cp = pltpu.make_async_copy(gw_hbm, small_buf.at[1], sem_small.at[2])
    wq_start(0, 0)
    x_cp.start(priority=0)
    for j in range(1, 2 * D1):
        wq_start(j >> 1, j & 1)
    wr_cp.start(priority=0)
    gw_cp.start(priority=0)
    a_buf[...] = jnp.zeros(a_buf.shape, f32)
    q_buf[...] = jnp.zeros(q_buf.shape, f32)
    h_buf[...] = jnp.zeros(h_buf.shape, f32)

    lane_id = jax.lax.broadcasted_iota(jnp.int32, (8, _LN), 1)
    diag = lane_id - jax.lax.broadcasted_iota(jnp.int32, (8, _LN), 0)

    def lane_sum(v):
        return jnp.broadcast_to(jnp.sum(v, axis=-1, keepdims=True), v.shape)

    def columns(v):
        return lane_sum(jnp.stack([jnp.where(diag == 8 * k, v, 0.0) for k in range(BT)]))

    def loop(lo, hi, body):
        def b(n, c):
            body(n)
            return c
        jax.lax.fori_loop(lo, hi, b, 0)

    def q_add(j):
        w = wq_buf[j].astype(f32)
        for r in range(WR):
            p = r * NW + j
            kb = _const_div(p, QB // 2, WR * NW)
            cb = 2 * p - QB * kb
            xc = [xc_buf[kb + WK * i] for i in range(WB // WR)]
            for jj in range(2):
                acc = q_buf[cb + jj]
                for i in range(WB // WR):
                    b = r + WR * i
                    acc = acc + w[8 * b:8 * b + 8, jj * _LN:(jj + 1) * _LN] * xc[i]
                q_buf[cb + jj] = acc

    def w_slot(j, u, job, nxt=False, nq=2):
        for i in range(2):
            wait_all(*wq_dst(j, i))
            if i < nq:
                wd_piece(u + i)
            if not nxt:
                wq_start(j + D1, i)
            elif i == 1:
                kv_start(k_hbm, j + D1 - NW)
        job()

    def x_job(t):
        if t == 0:
            x_cp.wait()
        xt = jnp.broadcast_to(x_buf[:, t * _LN:(t + 1) * _LN].astype(f32), (8, _LN))
        x8_buf[t] = xt
        xc_buf[pl.ds(t * BT, BT)] = columns(xt)

    def gate_job():
        wr_cp.wait()
        gw_cp.wait()
        wr = small_buf[0].astype(f32)
        gw = small_buf[1].astype(f32)
        r_acc = jnp.zeros((8, _LN), f32)
        g_acc = jnp.zeros((8, _LN), f32)
        for t in range(DB):
            xt = x8_buf[t]
            r_acc = r_acc + xt * jnp.broadcast_to(wr[t:t + 1, :], (8, _LN))
            g_acc = g_acc + xt * jnp.broadcast_to(gw[t:t + 1, :], (8, _LN))
        r_sel = jax.nn.sigmoid(lane_sum(r_acc))
        gate = jax.nn.sigmoid(lane_sum(g_acc))
        g_buf[0] = gate
        g_buf[1] = (1.0 - gate) * r_sel

    def row_sum(v):
        return jnp.broadcast_to(jnp.sum(v, axis=0, keepdims=True), (8, _LN))

    def q_fin(h):
        odd = h & 1
        cb = (3 * h) >> 1
        va, vb = row_sum(q_buf[cb]), row_sum(q_buf[cb + 1])
        vm = jnp.where(odd == 1, vb, va)
        lo, hi = diag - 64 * odd, diag + 64 * odd
        t = ([jnp.where(lo == 8 * r, va, 0.0) for r in range(8)]
             + [jnp.where(hi == 8 * r, vm, 0.0) for r in range(8, 16)]
             + [jnp.where(lo == 8 * r, vb, 0.0) for r in range(8)])
        qc_buf[pl.ds(h * RT, RT)] = lane_sum(jnp.stack(t))

    with scope("w0"):
        for t in range(DB):
            w_slot(t, t, functools.partial(x_job, t), nq=1)

        def two(j):
            q_add(j - DB)
            q_add(j)
        loop(DB, 2 * DB, lambda j: w_slot(j, 2 * j - DB, lambda: two(j)))

        def with_gate():
            gate_job()
            q_add(2 * DB)
        w_slot(2 * DB, 3 * DB, with_gate, nq=1)
    with scope("w1"):
        loop(2 * DB + 1, NW - D1, lambda j: w_slot(j, 2 * j - DB - 1, lambda: q_add(j)))
        jq = max(j for j in range(NW) for r in range(WR) if (r * NW + j) % (QB // 2) == 0) + 1
        assert NW - D1 <= jq < NW
        loop(NW - D1, jq, lambda j: w_slot(j, 2 * j - DB - 1, lambda: q_add(j), nxt=True))

        def with_fin():
            q_fin(0)
            q_add(jq)
        w_slot(jq, None, with_fin, nxt=True, nq=0)
        loop(jq + 1, NW, lambda j: w_slot(j, 2 * j - DB - 3, lambda: q_add(j), nxt=True))

    def lane_max(m):
        return jnp.broadcast_to(jnp.max(m, axis=-1, keepdims=True), (8, _LN))

    def score(t):
        p = (ring[t & (NC - 1)].astype(f32).reshape(RT // 4, 4, 8, _LN)
             * qc_buf[pl.ds((t >> 5) * RT, RT)].reshape(RT // 4, 4, 8, _LN))
        p = jnp.sum(p, axis=0)
        s = row_sum((p[0] + p[1]) + (p[2] + p[3]))
        s_buf[t] = s
        return s

    def k_slot(q0, nxt, t, m):
        c = t & (NC - 1)
        h = srl(t, 5)
        wait_all(ring.at[c], sem_ring.at[c])
        q0(NW + t)
        if nxt:
            kv_start(v_hbm, t + D1 - NS)
        else:
            kv_start(k_hbm, t + D1)
        m = jnp.maximum(jnp.where(c == 0, -jnp.inf, m), score(t))
        m_buf[h] = m

        @pl.when(c == JC)
        def _():
            hp = jnp.maximum(h - 1, 0)
            m_buf[hp] = lane_max(m_buf[hp])
            q_fin(jnp.minimum(h + 1, _HQ - 1))
        return m

    m = jnp.full((8, _LN), -jnp.inf, f32)
    lo = NW
    for hi, q0, nxt in ((S_WG, wd_start, False), (S_WU, wg_start, False), (S_WO, wu_start, False),
                        (S_V - D1, wo_start, False), (S_V, wo_start, True)):
        if nxt:
            e0 = jnp.exp((s_buf[0] - m_buf[0]) * scale)
        with scope("k%d" % lo):
            m = jax.lax.fori_loop(lo - NW, hi - NW, functools.partial(k_slot, q0, nxt), m)
        lo = hi

    def prob(n):
        return jnp.exp((s_buf[n] - m_buf[srl(n, 5)]) * scale)

    def pv_add(acc, e, c):
        return acc + ring[c].astype(f32).reshape(RT, 8, _LN) * e[None]

    def v_slot(h, c, st, job=None, tail=False):
        e, l, acc = st
        n = h * NC + c
        wait_all(ring.at[c], sem_ring.at[c])
        if tail:
            if TQ0 >= D1 - 1:
                tq0_start(c - D1)
            else:
                @pl.when(c - D1 < TQ0)
                def _():
                    tq0_start(c - D1)
        else:
            wo_start(S_V + n)
            kv_start(v_hbm, n + D1)
        acc = pv_add(acc, e, c)
        if job is not None:
            job()
        return prob(n + 1), l + e, acc

    def fin_job():
        acc_buf[...] = lane_sum(acc_buf[...])
        l_buf[...] = g_buf[0] / lane_sum(l_buf[...])
        m_buf[_HQ - 1] = lane_max(m_buf[_HQ - 1])

    def tiles_dot(buf, col, row, nt):
        w = buf[pl.ds(row, nt * BR), :].astype(f32).reshape(nt, DB, 8, _LN)
        return jnp.sum(w * col[:, None], axis=0)

    OJ = 4
    OT = RT // OJ

    def o_job(h, k):
        col = acc_buf[pl.ds(k * OT, OT)]
        a_buf[...] += (tiles_dot(wo_buf, col, mo((h * OJ + k) * (OT * BR), 16), OT)
                       * l_buf[...][None])

    def f_job(j):
        ch = srl(j, 1)
        up = jnp.bitwise_and(j, 1)
        x8 = jnp.concatenate([x8_buf[t] for t in range(DB)], axis=1).astype(bf16)
        t = jnp.dot(x8, wgu_buf[up, :, pl.ds(mo(ch * _LN, _LN), _LN)], preferred_element_type=f32)
        h_buf[ch] = jnp.where(up == 1, jax.nn.silu(h_buf[ch]), 1.0) * t

    def c_job(ch):
        hc_buf[pl.ds(ch * BT, BT)] = columns(h_buf[ch] * g_buf[1])

    def d_job(ch):
        a_buf[...] += tiles_dot(wd_buf, hc_buf[pl.ds(ch * BT, BT)], mo(ch * (BT * BR), 16), BT)

    DP = FB + 1
    assert DP + WD_B < _HQ and OC + 1 + OJ + 3 <= NC and OC + 1 + OJ <= D1

    def v_period(h, st):
        with scope("vper"):
            e, l, acc = st
            first = (h >= 1).astype(jnp.int32)
            nf = jnp.where(h < FB, 2, 0)
            nc = jnp.logical_and(h >= 1, h < DP).astype(jnp.int32)
            nd = jnp.logical_and(h >= DP, h < DP + WD_B).astype(jnp.int32)
            acc_buf[...] = acc
            l_buf[...] = l
            st = (e, jnp.zeros((8, _LN), f32), jnp.zeros((RT, 8, _LN), f32))
            st = jax.lax.fori_loop(0, OC, lambda c, st: v_slot(h, c, st), st)
            st = v_slot(h, jnp.int32(OC), st, fin_job)

            @pl.when(h >= 1)
            def _():
                wait_all(wo_buf.at[pl.ds(mo((h - 1) * (RT * BR), 64), RT * BR)], sem_wo.at[h - 1])
            c1 = OC + 1 + first * OJ
            st = jax.lax.fori_loop(
                OC + 1, c1, lambda c, st: v_slot(h, c, st, lambda: o_job(h - 1, c - OC - 1)), st)

            @pl.when(h == 0)
            def _():
                wait_all(wgu_buf, sem_gu.at[0])
            c2 = c1 + nf
            st = jax.lax.fori_loop(
                c1, c2, lambda c, st: v_slot(h, c, st, lambda: f_job(2 * h + c - c1)), st)
            c3 = c2 + nc
            st = jax.lax.fori_loop(c2, c3, lambda c, st: v_slot(h, c, st, lambda: c_job(h - 1)), st)

            @pl.when(h == DP)
            def _():
                wait_all(wd_buf.at[band_rows(0, TB)], sem_wd.at[0])
            c4 = c3 + nd
            st = jax.lax.fori_loop(c3, c4, lambda c, st: v_slot(h, c, st, lambda: d_job(h - DP)), st)
            st = jax.lax.fori_loop(c4, jnp.where(h == _HQ - 1, NC - D1, NC),
                                   lambda c, st: v_slot(h, c, st), st)
        return st
    st = (e0, jnp.ones((8, _LN), f32), jnp.zeros((RT, 8, _LN), f32))
    st = jax.lax.fori_loop(0, _HQ, v_period, st)

    def group_copy(i):
        sl = band_rows(*groups[i])
        return pltpu.make_async_copy(wd_hbm.at[sl], wd_buf.at[sl], sem_wd.at[1 + i])

    with scope("vlast"):
        for i in range(2, len(groups)):
            group_copy(i).start(priority=1)
        e, l, acc = jax.lax.fori_loop(
            NC - D1, NC - 1, lambda c, st: v_slot(_HQ - 1, c, st, tail=True), st)

    with scope("tail"):
        wait_all(wo_buf.at[pl.ds((_HQ - 1) * RT * BR, RT * BR)], sem_wo.at[_HQ - 1])
        gate = g_buf[0]
        inv = gate / lane_sum(l + e)
        base = []
        for cb in range(DB):
            xt = x8_buf[cb]
            base.append(((1.0 - gate) * (xt + xt * 0.0))[0:1])
        wait_all(ring.at[NC - 1], sem_ring.at[NC - 1])
        if TQ0 == D1:
            tq0_start(D1 - 1)
        col = lane_sum(pv_add(acc, e, NC - 1))
        a = a_buf[...] + tiles_dot(wo_buf, col, (_HQ - 1) * RT * BR, RT) * inv[None]
        for i in ORDER:
            b0, nb = groups[i]
            group_copy(i).wait()
            a = a + tiles_dot(wd_buf, hc_buf[pl.ds(b0, nb)], b0 * BR, nb)
        res = [base[cb] + jnp.sum(a[cb], axis=0, keepdims=True) for cb in range(DB)]
        o_ref[...] = jnp.concatenate(res, axis=1).astype(o_ref.dtype)


def _build(D1=16, SCOPES=False, TQ0=10, TQA=10, TAILP=(22, 10, 4, 2), ORDER=(0, 2, 3, 4, 5),
           OC=8, ST=256, JC=8):
    def fn(A_x, A_k_cache, A_v_cache, A_wq, A_wo, B_x, B_w_r, B_w_gate, B_w_up, B_w_down, gate_w):
        B, Sq, D = A_x.shape
        _, Hkv, SK, Dh = A_k_cache.shape
        assert B == 1 and Sq == 1 and Hkv == _HQ and Dh == _DH
        W = min(4096, max(256, SK // 4))
        F = B_w_gate.shape[1]
        n_rows = _HQ * _DH
        NC = W // _LN
        DB, FB = D // _LN, F // _LN
        bf16, f32 = jnp.bfloat16, jnp.float32

        def tiles(w, st=1):
            r, c = w.shape
            t = w.reshape(r // 8, 8, c // _LN, _LN).transpose(0, 2, 1, 3)
            n = (r // 8) * (c // _LN) // st
            return t.reshape(n, st, 8, _LN).transpose(0, 2, 1, 3).reshape(n * 8, st * _LN)

        x = A_x.reshape(1, D)
        kt = jnp.swapaxes(A_k_cache, 2, 3).reshape(n_rows, SK)
        vt = jnp.swapaxes(A_v_cache, 2, 3).reshape(n_rows, SK)
        wr = B_w_r.reshape(DB, _LN)
        gw = gate_w.reshape(DB, _LN)
        wq = tiles(A_wq, ST)

        any_spec = pl.BlockSpec(memory_space=pl.ANY)
        out = pl.pallas_call(
            functools.partial(_kernel, D1=D1, W=W, SK=SK, D=D, F=F, ST=ST, SCOPES=SCOPES, TQ0=TQ0,
                              TQA=TQA, TAILP=TAILP, ORDER=ORDER, OC=OC, JC=JC),
            in_specs=[any_spec] * 10,
            out_specs=pl.BlockSpec(memory_space=pltpu.VMEM),
            out_shape=jax.ShapeDtypeStruct((1, D), bf16),
            scratch_shapes=[
                pltpu.VMEM((1, D), bf16),
                pltpu.VMEM((2, DB, _LN), bf16),
                pltpu.VMEM((ST // 2, wq.shape[0], 2 * _LN), bf16),
                pltpu.VMEM((2, D, F), bf16),
                pltpu.VMEM((n_rows * DB, _LN), bf16),
                pltpu.VMEM((F * DB, _LN), bf16),
                pltpu.VMEM((NC, _DH, _LN), bf16),
                pltpu.VMEM((DB, 8, _LN), f32),
                pltpu.VMEM((D // 8, 8, _LN), f32),
                pltpu.VMEM((2, 8, _LN), f32),
                pltpu.VMEM((n_rows // _LN, 8, _LN), f32),
                pltpu.VMEM((n_rows // 8, 8, _LN), f32),
                pltpu.VMEM((_HQ * NC, 8, _LN), f32),
                pltpu.VMEM((_HQ, 8, _LN), f32),
                pltpu.VMEM((_DH // 8, 8, _LN), f32),
                pltpu.VMEM((8, _LN), f32),
                pltpu.VMEM((FB, 8, _LN), f32),
                pltpu.VMEM((F // 8, 8, _LN), f32),
                pltpu.VMEM((DB, 8, _LN), f32),
                pltpu.SemaphoreType.DMA((3,)),
                pltpu.SemaphoreType.DMA((2 * D1,)),
                pltpu.SemaphoreType.DMA((1,)),
                pltpu.SemaphoreType.DMA((_HQ,)),
                pltpu.SemaphoreType.DMA((3 + len(TAILP),)),
                pltpu.SemaphoreType.DMA((NC,)),
            ],
            compiler_params=_compiler_params(vmem_limit_bytes=100 * 1024 * 1024,
                                             disable_bounds_checks=True,
                                             disable_semaphore_checks=True),
        )(x, kt, vt, wq, tiles(A_wo), wr, B_w_gate, B_w_up, tiles(B_w_down), gw)
        return out.reshape(B, Sq, D)
    return fn


@jax.jit
def pallas_gated_mix__sliding_block_cached__moe_arch_mod__decode_kernel(
    A_x: jax.Array,
    A_k_cache: jax.Array,
    A_v_cache: jax.Array,
    A_wq: jax.Array,
    A_wo: jax.Array,
    B_x: jax.Array,
    B_w_r: jax.Array,
    B_w_gate: jax.Array,
    B_w_up: jax.Array,
    B_w_down: jax.Array,
    gate_w: jax.Array,
):
    return _build()(A_x, A_k_cache, A_v_cache, A_wq, A_wo, B_x, B_w_r,
                    B_w_gate, B_w_up, B_w_down, gate_w)
```
